```python
import jax
import jax.numpy as jnp

def _softmax(x, axis=-1):
    return jax.nn.softmax(x, axis=axis)

def _gelu(x):
    return jax.nn.gelu(x, approximate=True)

def _silu(x):
    return jax.nn.silu(x)

def _sigmoid(x):
    return jax.nn.sigmoid(x)

def _layernorm(x, axis=-1, eps=1e-05):
    m = jnp.mean(x, axis=axis, keepdims=True)
    v = jnp.var(x, axis=axis, keepdims=True)
    return (x - m) / jnp.sqrt(v + eps)

def _scatter_add(tgt, idx, src, axis=0):
    return tgt.at[idx].add(src)

def _segment_sum(src, seg, n):
    return jax.ops.segment_sum(src, seg, n)

class _Rng:

    def __init__(self, key):
        self._k = key

    def _next(self):
        self._k, sub = jax.random.split(self._k)
        return sub

    def normal(self, shape):
        return jax.random.normal(self._next(), shape, dtype=jnp.bfloat16)

    def randint(self, lo, hi, shape):
        return jax.random.randint(self._next(), shape, lo, hi, dtype=jnp.int32)

    def uniform(self, shape, lo=0.0, hi=1.0):
        return jax.random.uniform(self._next(), shape, jnp.bfloat16, lo, hi)

    def permutation(self, n):
        return jax.random.permutation(self._next(), n)
kernel_name = 'concat_heads__memory_aug_recurrent_mem_tr__spectral_gfnet__prompt'

def setup_inputs():
    _rng = _Rng(jax.random.key(int.from_bytes(__import__("os").urandom(4), "little")))
    _w = lambda a: (lambda t: t.astype(jnp.bfloat16) if jnp.issubdtype(t.dtype, jnp.floating) else t)(jnp.asarray(a))

    def _A_setup():
        B, S, Dm = (1, 2048, 1024)
        H, Dh = (32, 128)
        M, seg = (8, 32)
        seg = min(seg, S)
        S = S // seg * seg
        return {'x': _w((lambda *s: _rng.normal(s) * 0.05)(B, S, Dm)), 'mem0': _w((lambda *s: _rng.normal(s) * 0.05)(B, M, Dm)), 'Wq': _w((lambda *s: _rng.normal(s) * 0.05)(Dm, H, Dh) * Dm ** (-0.5)), 'Wk': _w((lambda *s: _rng.normal(s) * 0.05)(Dm, H, Dh) * Dm ** (-0.5)), 'Wv': _w((lambda *s: _rng.normal(s) * 0.05)(Dm, H, Dh) * Dm ** (-0.5)), 'Wo': _w((lambda *s: _rng.normal(s) * 0.05)(H, Dh, Dm) * (H * Dh) ** (-0.5)), 'seg_len': seg}
    _A_in = _A_setup()

    def _B_setup():
        B, S, D = (1, 2048, 1024)
        Df = D // 2 + 1
        return {'x': _w((lambda *s: _rng.normal(s) * 0.05)(B, S, D)), 'w_r': _w((lambda *s: _rng.normal(s) * 0.05)(S, Df) * 0.02), 'w_i': _w((lambda *s: _rng.normal(s) * 0.05)(S, Df) * 0.02)}
    _B_in = _B_setup()
    return {'A_x': _A_in['x'], 'A_mem0': _A_in['mem0'], 'A_Wq': _A_in['Wq'], 'A_Wk': _A_in['Wk'], 'A_Wv': _A_in['Wv'], 'A_Wo': _A_in['Wo'], 'A_seg_len': _A_in['seg_len'], 'B_x': _B_in['x'], 'B_w_r': _B_in['w_r'], 'B_w_i': _B_in['w_i']}

def reference(A_x, A_mem0, A_Wq, A_Wk, A_Wv, A_Wo, A_seg_len, B_x, B_w_r, B_w_i):

    def _A_ref(x, mem0, Wq, Wk, Wv, Wo, seg_len):
        B, S, Dm = x.shape
        H, Dh = (Wq.shape[1], Wq.shape[2])
        M = mem0.shape[1]
        scale = Dh ** (-0.5)
        n_seg = S // seg_len
        L = M + seg_len
        idx = jnp.arange(L)
        mask = (idx[:, None] < M) | (idx[:, None] >= idx[None, :])
        mem = mem0
        outs = []
        for s in range(n_seg):
            xs = x[:, s * seg_len:(s + 1) * seg_len, :].copy()
            h = jnp.concatenate([mem, xs], axis=1)
            q = jnp.einsum('btd,dhe->bhte', h, Wq)
            k = jnp.einsum('btd,dhe->bhte', h, Wk)
            v = jnp.einsum('btd,dhe->bhte', h, Wv)
            scores = jnp.einsum('bhqe,bhke->bhqk', q, k) * scale
            scores = jnp.where(mask[None, None], scores, -1000000000.0)
            p = _softmax(scores, axis=-1)
            o = jnp.einsum('bhqk,bhke->bhqe', p, v)
            o = jnp.einsum('bhte,hed->btd', o, Wo)
            mem = o[:, :M, :].copy()
            outs.append(o[:, M:, :])
        return jnp.concatenate(outs, axis=1)

    def _B_ref(x, w_r, w_i):
        B, S, D = x.shape
        X = (lambda x, axes=(-2, -1): jnp.fft.rfft2(x.astype(jnp.float32), axes=axes))(x, axes=(-2, -1))
        W = w_r + 1j * w_i
        X = X * W
        y = (lambda x, s, axes=(-2, -1): jnp.fft.irfft2(x, s=s, axes=axes).astype(jnp.bfloat16))(X, (S, D), axes=(-2, -1))
        return y
    a = _A_ref(A_x, A_mem0, A_Wq, A_Wk, A_Wv, A_Wo, A_seg_len)
    b = _B_ref(B_x, B_w_r, B_w_i)
    return jnp.concatenate([a, b], axis=-1)
```

```python
import functools

import jax
import jax.numpy as jnp
import numpy as np
from jax import lax
import jax.experimental.pallas as pl
import jax.experimental.pallas.tpu as pltpu

f32, bf16, u32 = jnp.float32, jnp.bfloat16, jnp.uint32

S, D = 2048, 1024
H, DH, M, SEG = 32, 128, 8, 32
L = M + SEG
NSEG = S // SEG
R, P = 16, 128
NT = D // 2 // 128


def _pack_rows(a):
    b = a.astype(bf16).view(np.uint16).astype(np.uint32)
    w = b[0::2] | (b[1::2] << 16)
    return np.ascontiguousarray(w.reshape(w.shape[0], -1, 128).transpose(1, 0, 2))


_RT = float(np.sqrt(0.5))


def _split8(x):
    a0, a1, b0, b1 = x[0] + x[4], x[0] - x[4], x[2] + x[6], x[2] - x[6]
    c0, c1, d0, d1 = x[1] + x[5], x[1] - x[5], x[3] + x[7], x[3] - x[7]
    e, f = a0 + b0, c0 + d0
    u, v = (c1 - d1) * _RT, (c1 + d1) * _RT
    return [e + f, e - f, a1 + u, b1 + v, a0 - b0, c0 - d0, a1 - u, b1 - v]


def _merge8(y):
    e, f = y[0] + y[1], y[0] - y[1]
    a0, b0, c0, d0 = e + y[4], e - y[4], f + y[5], f - y[5]
    a1, b1 = y[2] + y[6], y[3] + y[7]
    u, v = (y[2] - y[6]) * _RT, (y[3] - y[7]) * _RT
    c1, d1 = u + v, v - u
    return [a0 + a1, c0 + c1, b0 + b1, d0 + d1, a0 - a1, c0 - c1, b0 - b1, d0 - d1]


_GROUPS = ((0, 4), (1, 7), (2, 6), (3, 5))


@functools.lru_cache(maxsize=None)
def _constants():
    basis = np.stack(_split8(list(np.eye(8))))
    d = np.arange(D)[None, :]
    mf, mi = [], []
    for g, ks in enumerate(_GROUPS):
        kd = np.concatenate([k1 + 8 * np.arange(64) for k1 in ks])[:, None]
        ang = 2.0 * np.pi * ((d * kd) % D) / D
        rows = np.concatenate([np.cos(ang), -np.sin(ang)], axis=0)
        wgt = np.full((2 * 128,), 2.0)
        if g == 0:
            rows[128] = 1.0 - 2.0 * (np.arange(D) % 2)
            wgt[0] = wgt[128] = 1.0
        bg = basis[2 * g:2 * g + 2]
        rows = rows.reshape(256, 8, 128)
        m = np.einsum("oad,as->osd", rows, np.linalg.pinv(bg))
        assert np.abs(np.einsum("osd,sa->oad", m, bg) - rows).max() < 1e-9
        m = m.reshape(256, 256)
        mf.append(m)
        mi.append(_pack_rows(m * wgt[:, None] / (S * D)))
    k2 = np.arange(P)[None, :]
    n2 = np.arange(P)[:, None]
    gf = []
    for n1 in range(R):
        a = 2.0 * np.pi * ((k2 * (n1 + R * n2)) % S) / S
        gr, gi = np.cos(a), -np.sin(a)
        gf.append(np.block([[gr, gi], [-gi, gr]]))
    gf = np.stack(gf)
    return (np.stack(mf).astype(bf16), np.concatenate(mi), np.concatenate([_pack_rows(g) for g in gf]),
            gf.astype(bf16))


def _fft16(xs, sign):
    def bf4(a, b, c, d):
        s0 = (a[0] + c[0], a[1] + c[1])
        s1 = (a[0] - c[0], a[1] - c[1])
        s2 = (b[0] + d[0], b[1] + d[1])
        s3 = (b[0] - d[0], b[1] - d[1])
        p = (s1[0] - s3[1], s1[1] + s3[0])
        m = (s1[0] + s3[1], s1[1] - s3[0])
        o1, o3 = (p, m) if sign > 0 else (m, p)
        return [(s0[0] + s2[0], s0[1] + s2[1]), o1, (s0[0] - s2[0], s0[1] - s2[1]), o3]

    def tw(x, e):
        e = e % 16
        if e == 0:
            return x
        if e == 4:
            return (-x[1], x[0]) if sign > 0 else (x[1], -x[0])
        c = np.float32(np.cos(2 * np.pi * e / 16))
        s = np.float32(sign * np.sin(2 * np.pi * e / 16))
        if e == 2:
            return ((x[0] - x[1]) * c, (x[0] + x[1]) * c) if sign > 0 else ((x[0] + x[1]) * c, (x[1] - x[0]) * c)
        if e == 6:
            return ((x[0] + x[1]) * c, (x[1] - x[0]) * c) if sign > 0 else ((x[0] - x[1]) * c, (x[0] + x[1]) * c)
        return (x[0] * c - x[1] * s, x[0] * s + x[1] * c)

    inner = [bf4(xs[b], xs[4 + b], xs[8 + b], xs[12 + b]) for b in range(4)]
    out = [None] * 16
    for c in range(4):
        o = bf4(*[tw(inner[b][c], b * c) for b in range(4)])
        for e in range(4):
            out[c + 4 * e] = o[e]
    return out


def _nt(a, b):
    return lax.dot_general(a, b, (((1,), (1,)), ((), ())), preferred_element_type=f32)


def _tiles(ref, i):
    return jnp.concatenate([pltpu.bitcast(ref[i], bf16), pltpu.bitcast(ref[i + 1], bf16)], axis=1)


def _kernel(ax_hbm, mem_hbm, wq_hbm, wk_hbm, wv_hbm, wo_hbm, bx_hbm, wr_hbm, wi_hbm, wrn_ref, win_ref,
            mf_hbm, mi_hbm, gf_hbm, gi_hbm, out_hbm,
            wqkv, wo, ax, oa, bx, mf, mi, gf, gi, wr, wi, tp, mem_ref,
            hbuf, obuf, qkv, pbuf, sem_bx, sem, sem_out):
    bx32 = bx_hbm.bitcast(u32)
    out32 = out_hbm.bitcast(u32)

    def bx_copy(j):
        return pltpu.make_async_copy(bx32.at[:, j, :], bx.at[j], sem_bx.at[j])

    def y_copy(j):
        return pltpu.make_async_copy(bx.at[j], out32.at[:, j, pl.ds(D, D)], sem.at[10])

    mf_copy = pltpu.make_async_copy(mf_hbm, mf, sem.at[0])
    gf_copy = pltpu.make_async_copy(gf_hbm, gf, sem.at[1])
    gi_copy = pltpu.make_async_copy(gi_hbm, gi, sem.at[2])
    mi_copy = pltpu.make_async_copy(mi_hbm, mi, sem.at[3])
    ax_copy = pltpu.make_async_copy(ax_hbm, ax, sem.at[4])
    mem_copy = pltpu.make_async_copy(mem_hbm, mem_ref, sem.at[11])
    w_copies = [pltpu.make_async_copy(src.at[pl.ds(0, D // 2), pl.ds(k1 * P, P)].bitcast(u32), dst.at[k1], sem.at[5])
                for src, dst in ((wr_hbm, wr), (wi_hbm, wi)) for k1 in range(R)]
    qkv_copies = []
    for m, src in enumerate((wq_hbm, wk_hbm, wv_hbm)):
        s32 = src.bitcast(u32)
        qkv_copies.append([pltpu.make_async_copy(s32.at[:, j, :], wqkv.at[m * (H // 2) + j], sem.at[6 + m])
                           for j in range(H // 2)])
    wo32 = wo_hbm.bitcast(u32)
    wo_copies = [pltpu.make_async_copy(wo32.at[:, pl.ds(c * 128, 128)], wo.at[c], sem.at[9]) for c in range(D // 128)]

    bx_copy(0).start()
    mf_copy.start()
    gf_copy.start()
    for j in range(1, R // 2):
        bx_copy(j).start()
    for cp in w_copies:
        cp.start()
    gi_copy.start()
    mi_copy.start()
    mem_copy.start()
    for cps in qkv_copies:
        for cp in cps:
            cp.start()
    ax_copy.start()
    for cp in wo_copies:
        cp.start()

    def unpack(w, par):
        return pltpu.bitcast((w << 16) if par == 0 else (w & jnp.uint32(0xFFFF0000)), f32)

    mf_copy.wait()
    gf_copy.wait()
    row0 = lax.broadcasted_iota(jnp.int32, (8, 128), 0) == 0

    def fwd(j, carry):
        bx_copy(j).wait()
        zs = []
        for par in range(2):
            sig = _split8([unpack(bx[j, :, t * 128:(t + 1) * 128], par) for t in range(8)])
            zs.append([_nt(mf[g], jnp.concatenate([sig[2 * g].astype(bf16), sig[2 * g + 1].astype(bf16)], axis=1))
                       for g in range(NT)])
        for par in range(2):
            z = zs[par]
            head = z[0][128:136]
            re = [zg[:128] for zg in z] + [jnp.where(row0, head, 0.0)]
            im = [jnp.where(row0, 0.0, head), z[0][136:]] + [zg[128:] for zg in z[1:]] + [jnp.zeros((8, 128), f32)]
            lhs = jnp.concatenate([jnp.concatenate(re, axis=0), jnp.concatenate(im, axis=0)], axis=1)
            n1 = 2 * j + par
            tp[n1] = jnp.dot(lhs, _tiles(gf, 2 * n1), preferred_element_type=f32)
        return carry

    lax.fori_loop(0, R // 2, fwd, 0)

    for cp in w_copies:
        cp.wait()

    def filt(r0, w_of):
        xs = _fft16([(tp[n1, pl.ds(r0, 8), :P], tp[n1, pl.ds(r0, 8), P:]) for n1 in range(R)], -1)
        ys = []
        for k1, (ur, ui) in enumerate(xs):
            a, b = w_of(k1)
            ys.append((ur * a - ui * b, ur * b + ui * a))
        for n1, (yr, yi) in enumerate(_fft16(ys, 1)):
            tp[n1, pl.ds(r0, 8), :P] = yr
            tp[n1, pl.ds(r0, 8), P:] = yi

    for g, ks in enumerate(_GROUPS):
        for half, k1d in enumerate(ks):
            def body(i, carry, base=g * 128 + half * 64, k1d=k1d):
                def w_of(k1):
                    rows = pl.ds(32 * i + k1d // 2, 8, stride=4)
                    return (unpack(wr[k1, rows, :], k1d % 2),
                            unpack(wi[k1, rows, :], k1d % 2))
                filt(pl.multiple_of(base + 8 * i, 8), w_of)
                return carry
            lax.fori_loop(0, 8, body, 0)
    filt(D // 2, lambda k1: (jnp.where(row0, wrn_ref[:, k1 * P:(k1 + 1) * P].astype(f32), 0.0),
                             jnp.where(row0, win_ref[:, k1 * P:(k1 + 1) * P].astype(f32), 0.0)))

    gi_copy.wait()
    mi_copy.wait()
    lane0 = lax.broadcasted_iota(jnp.int32, (P, 128), 1) == 0

    def inv(j, carry):
        ts = []
        for par in range(2):
            n1 = 2 * j + par
            ts.append([_nt(gi[n1], tp[n1, t * 128:(t + 1) * 128, :].astype(bf16)) for t in range(NT)])
        for par in range(2):
            n1 = 2 * j + par
            ny = jnp.concatenate([tp[n1, D // 2:, :], jnp.zeros((120, 2 * P), f32)], axis=0)
            ts[par].append(_nt(gi[n1, :P, :], ny.astype(bf16)))
        sig = [[], []]
        for g in range(NT):
            rows = []
            for par in range(2):
                t = ts[par][g]
                ti = jnp.where(lane0, ts[par][NT], t[P:]) if g == 0 else t[P:]
                rows.append(jnp.concatenate([t[:P], ti], axis=1))
            o = jnp.dot(jnp.concatenate(rows, axis=0), _tiles(mi, 2 * g), preferred_element_type=f32)
            for par in range(2):
                sig[par] += [o[par * P:(par + 1) * P, :128], o[par * P:(par + 1) * P, 128:]]
        y0, y1 = _merge8(sig[0]), _merge8(sig[1])
        for t in range(8):
            bx[j, :, t * 128:(t + 1) * 128] = pltpu.pack_elementwise([y0[t], y1[t]], packed_dtype=bf16)
        y_copy(j).start()
        return carry

    lax.fori_loop(0, R // 2, inv, 0)

    for m in range(3):
        for cp in qkv_copies[m]:
            cp.wait()

        def split(g, carry, m=m):
            j = m * (H // 2) + g // 4
            base = pl.multiple_of((g % 4) * 256, 256)
            ev = [wqkv[j, pl.ds(base + 16 * i, 8, stride=2), :] for i in range(16)]
            od = [wqkv[j, pl.ds(base + 16 * i + 1, 8, stride=2), :] for i in range(16)]
            for i in range(16):
                wqkv[j, pl.ds(base + 16 * i, 8), :] = (ev[i] & 0xFFFF) | (od[i] << 16)
                wqkv[j, pl.ds(base + 16 * i + 8, 8), :] = (ev[i] >> 16) | (od[i] & jnp.uint32(0xFFFF0000))
            return carry

        lax.fori_loop(0, (H // 2) * 4, split, 0)

    ax_copy.wait()
    for cp in wo_copies:
        cp.wait()
    mem_copy.wait()
    hbuf[0:M, :] = mem_ref[...].astype(f32)
    row = lax.broadcasted_iota(jnp.int32, (L, L), 0)
    col = lax.broadcasted_iota(jnp.int32, (L, L), 1)
    mask = (row < M) | (row >= col)
    scale = np.float32(DH ** -0.5)
    wsplit = wqkv.reshape(3 * (H // 2), D // 16, 16, 128)

    def out_copy(s):
        return pltpu.make_async_copy(oa.at[pl.ds(2 * s, 2)], out_hbm.at[pl.ds(2 * s, 2), :, pl.ds(0, D)], sem_out.at[0])

    def seg(s, carry):
        r0 = pl.multiple_of(s * SEG, SEG)
        hbuf[M:L, :] = ax[pl.ds(r0, SEG), :].astype(f32)

        def proj(h):
            for m in range(3):
                w = wsplit[m * (H // 2) + h // 2, :, 8 * (h % 2):8 * (h % 2) + 8, :].reshape(D // 2, 128)
                qkv[h % 4, m] = jnp.dot(hbuf[...], pltpu.bitcast(w, bf16), preferred_element_type=f32)

        def scores(h):
            sc = lax.dot_general(qkv[h % 4, 0], qkv[h % 4, 1], (((1,), (1,)), ((), ())),
                                 preferred_element_type=f32) * scale
            sc = jnp.where(mask, sc, -1e9)
            e = jnp.exp(sc - jnp.max(sc, axis=-1, keepdims=True))
            pbuf[h % 4] = e / jnp.sum(e, axis=-1, keepdims=True)

        def pv(h):
            obuf[:, DH * h:DH * (h + 1)] = jnp.dot(pbuf[h % 4], qkv[h % 4, 2], preferred_element_type=f32)

        def oproj(c, h0, h1):
            return jnp.dot(obuf[:, DH * h0:DH * h1], pltpu.bitcast(wo[c, 64 * h0:64 * h1, :], bf16),
                           preferred_element_type=f32)

        def finish(c, o):
            hbuf[0:M, 128 * c:128 * (c + 1)] = o[0:M].astype(bf16).astype(f32)
            oa[pl.ds(2 * s, 2), :, 128 * c:128 * (c + 1)] = o[M:L].astype(bf16).reshape(2, R, 128)

        for h in range(H):
            proj(h)
            if h >= 1:
                scores(h - 1)
            if h >= 2:
                pv(h - 2)
        scores(H - 1)
        a0 = oproj(0, 0, 16)
        pv(H - 2)
        a1 = oproj(1, 0, 16)
        a2 = oproj(2, 0, 16)
        pv(H - 1)
        a3 = oproj(3, 0, 16)
        for c, a in enumerate((a0, a1, a2, a3)):
            finish(c, a + oproj(c, 16, 32))
        for c in range(4, 8):
            finish(c, oproj(c, 0, 32))
        out_copy(s).start()
        return carry

    lax.fori_loop(0, NSEG, seg, 0)

    def drain(s, carry):
        out_copy(s).wait()
        return carry

    lax.fori_loop(0, NSEG, drain, 0)
    for j in range(R // 2):
        y_copy(j).wait()


@functools.partial(jax.jit, static_argnames=("A_seg_len",))
def pallas_concat_heads__memory_aug_recurrent_mem_tr__spectral_gfnet__prompt_kernel(
    A_x, A_mem0, A_Wq, A_Wk, A_Wv, A_Wo, A_seg_len, B_x, B_w_r, B_w_i,
):
    assert A_seg_len == SEG and A_x.shape == (1, S, D) and B_x.shape == (1, S, D)
    mf, mi, gf, gi = _constants()
    hbm = pl.BlockSpec(memory_space=pltpu.HBM)
    nyq = pl.BlockSpec((8, S), lambda i: (D // 16, 0))
    wr, wi = B_w_r.T, B_w_i.T
    out = pl.pallas_call(
        _kernel,
        out_shape=jax.ShapeDtypeStruct((P, R, 2 * D), bf16),
        grid=(1,),
        in_specs=[hbm] * 9 + [nyq, nyq] + [hbm] * 4,
        out_specs=hbm,
        scratch_shapes=[
            pltpu.VMEM((3 * H // 2, D, 128), u32),
            pltpu.VMEM((D // 128, H * DH // 2, 128), u32),
            pltpu.VMEM((S, D), bf16),
            pltpu.VMEM((P, R, D), bf16),
            pltpu.VMEM((R // 2, P, D), u32),
            pltpu.VMEM((NT, 256, 256), bf16),
            pltpu.VMEM((2 * NT, 128, 128), u32),
            pltpu.VMEM((2 * R, P, 128), u32),
            pltpu.VMEM((R, 2 * P, 2 * P), bf16),
            pltpu.VMEM((R, D // 4, P), u32),
            pltpu.VMEM((R, D // 4, P), u32),
            pltpu.VMEM((R, D // 2 + 8, 2 * P), f32),
            pltpu.VMEM((M, D), bf16),
            pltpu.VMEM((L, D), f32),
            pltpu.VMEM((L, H * DH), f32),
            pltpu.VMEM((4, 3, L, DH), f32),
            pltpu.VMEM((4, L, L), f32),
            pltpu.SemaphoreType.DMA((R // 2,)),
            pltpu.SemaphoreType.DMA((12,)),
            pltpu.SemaphoreType.DMA((1,)),
        ],
        compiler_params=pltpu.CompilerParams(vmem_limit_bytes=110 * 2**20),
        name="rmt_gfnet",
    )(A_x.reshape(S, D), A_mem0.reshape(M, D), A_Wq, A_Wk, A_Wv, A_Wo.reshape(H * DH, D),
      B_x.reshape(P, R, D), wr, wi, wr, wi, mf, mi, gf, gi)
    return out.reshape(1, S, 2 * D)
```

```python
import functools

import jax
import jax.numpy as jnp
import numpy as np
from jax import lax
import jax.experimental.pallas as pl
import jax.experimental.pallas.tpu as pltpu

f32, bf16, u32 = jnp.float32, jnp.bfloat16, jnp.uint32

S, D = 2048, 1024
H, DH, M, SEG = 32, 128, 8, 32
L = M + SEG
NSEG = S // SEG
R, P = 16, 128
NT = D // 2 // 128


_RT = float(np.sqrt(0.5))


def _split8(x):
    a0, a1, b0, b1 = x[0] + x[4], x[0] - x[4], x[2] + x[6], x[2] - x[6]
    c0, c1, d0, d1 = x[1] + x[5], x[1] - x[5], x[3] + x[7], x[3] - x[7]
    e, f = a0 + b0, c0 + d0
    u, v = (c1 - d1) * _RT, (c1 + d1) * _RT
    return [e + f, e - f, a1 + u, b1 + v, a0 - b0, c0 - d0, a1 - u, b1 - v]


def _merge8(y):
    e, f = y[0] + y[1], y[0] - y[1]
    a0, b0, c0, d0 = e + y[4], e - y[4], f + y[5], f - y[5]
    a1, b1 = y[2] + y[6], y[3] + y[7]
    u, v = (y[2] - y[6]) * _RT, (y[3] - y[7]) * _RT
    c1, d1 = u + v, v - u
    return [a0 + a1, c0 + c1, b0 + b1, d0 + d1, a0 - a1, c0 - c1, b0 - b1, d0 - d1]


_GROUPS = ((0, 4), (1, 7), (2, 6), (3, 5))


@functools.lru_cache(maxsize=None)
def _constants():
    basis = np.stack(_split8(list(np.eye(8))))
    d = np.arange(D)[None, :]
    mf = []
    for g, ks in enumerate(_GROUPS):
        kd = np.sort(np.concatenate([k1 + 8 * np.arange(64) for k1 in ks]))[:, None]
        ang = 2.0 * np.pi * ((d * kd) % D) / D
        rows = np.concatenate([np.cos(ang), -np.sin(ang)], axis=0)
        if g == 0:
            rows[128] = 1.0 - 2.0 * (np.arange(D) % 2)
        bg = basis[2 * g:2 * g + 2]
        rows = rows.reshape(256, 8, 128)
        m = np.einsum("oad,as->osd", rows, np.linalg.pinv(bg))
        assert np.abs(np.einsum("osd,sa->oad", m, bg) - rows).max() < 1e-9
        mf.append(m.reshape(256, 256))
    k2 = np.arange(P)[None, :]
    a = 2.0 * np.pi * ((np.arange(P)[:, None] * k2) % P) / P
    t = 2.0 * np.pi * (np.repeat(np.arange(R), 8)[:, None] * k2) / S
    tab = np.stack([np.cos(a), -np.sin(a), np.cos(t) * 2.0 ** -10, -np.sin(t) * 2.0 ** -10])
    return np.stack(mf).astype(bf16), tab.astype(np.float32)


def _fft16(xs, sign):
    def bf4(a, b, c, d):
        s0 = (a[0] + c[0], a[1] + c[1])
        s1 = (a[0] - c[0], a[1] - c[1])
        s2 = (b[0] + d[0], b[1] + d[1])
        s3 = (b[0] - d[0], b[1] - d[1])
        p = (s1[0] - s3[1], s1[1] + s3[0])
        m = (s1[0] + s3[1], s1[1] - s3[0])
        o1, o3 = (p, m) if sign > 0 else (m, p)
        return [(s0[0] + s2[0], s0[1] + s2[1]), o1, (s0[0] - s2[0], s0[1] - s2[1]), o3]

    def tw(x, e):
        e = e % 16
        if e == 0:
            return x
        if e == 4:
            return (-x[1], x[0]) if sign > 0 else (x[1], -x[0])
        c = np.float32(np.cos(2 * np.pi * e / 16))
        s = np.float32(sign * np.sin(2 * np.pi * e / 16))
        if e == 2:
            return ((x[0] - x[1]) * c, (x[0] + x[1]) * c) if sign > 0 else ((x[0] + x[1]) * c, (x[1] - x[0]) * c)
        if e == 6:
            return ((x[0] + x[1]) * c, (x[1] - x[0]) * c) if sign > 0 else ((x[0] - x[1]) * c, (x[0] + x[1]) * c)
        return (x[0] * c - x[1] * s, x[0] * s + x[1] * c)

    inner = [bf4(xs[b], xs[4 + b], xs[8 + b], xs[12 + b]) for b in range(4)]
    out = [None] * 16
    for c in range(4):
        o = bf4(*[tw(inner[b][c], b * c) for b in range(4)])
        for e in range(4):
            out[c + 4 * e] = o[e]
    return out


def _nt(a, b):
    return lax.dot_general(a, b, (((1,), (1,)), ((), ())), preferred_element_type=f32)


def _kernel(ax_hbm, mem_hbm, wq_hbm, wk_hbm, wv_hbm, wo_hbm, bx_hbm, wr_hbm, wi_hbm, wrn_ref, win_ref,
            mf_hbm, tab_hbm, out_hbm,
            wqkv, wo, ax, oa, bx, mf, tab, gf, wr, wi, tp, mem_ref,
            hbuf, obuf, qkv, pbuf, part, sem_bx, sem_qkv, sem_wo, sem, sem_out):
    bx32 = bx_hbm.bitcast(u32)
    out32 = out_hbm.bitcast(u32)

    def bx_copy(j):
        return pltpu.make_async_copy(bx32.at[:, j, :], bx.at[j], sem_bx.at[j])

    def y_copy(j):
        return pltpu.make_async_copy(bx.at[j], out32.at[:, j, pl.ds(D, D)], sem.at[10])

    mf_copy = pltpu.make_async_copy(mf_hbm, mf, sem.at[0])
    tab_copy = pltpu.make_async_copy(tab_hbm, tab, sem.at[1])
    ax0_copy = pltpu.make_async_copy(ax_hbm.at[pl.ds(0, SEG), :], ax.at[pl.ds(0, SEG), :], sem.at[2])
    ax_copy = pltpu.make_async_copy(ax_hbm.at[pl.ds(SEG, S - SEG), :], ax.at[pl.ds(SEG, S - SEG), :], sem.at[3])
    mem_copy = pltpu.make_async_copy(mem_hbm, mem_ref, sem.at[11])
    w_copies = [pltpu.make_async_copy(src.at[pl.ds(0, D // 2), pl.ds(k1 * P, P)].bitcast(u32), dst.at[k1], sem.at[5])
                for src, dst in ((wr_hbm, wr), (wi_hbm, wi)) for k1 in range(R)]

    def qkv_copies(j):
        return [pltpu.make_async_copy(src.bitcast(u32).at[:, j, :], wqkv.at[m * (H // 2) + j], sem_qkv.at[j])
                for m, src in enumerate((wq_hbm, wk_hbm, wv_hbm))]

    wo32 = wo_hbm.bitcast(u32)
    wo_copies = [pltpu.make_async_copy(wo32.at[:, pl.ds(c * 128, 128)], wo.at[c], sem_wo.at[c]) for c in range(D // 128)]

    mf_copy.start()
    bx_copy(0).start()
    tab_copy.start()
    for j in range(1, R // 2):
        bx_copy(j).start()
    for cp in w_copies:
        cp.start()
    mem_copy.start()
    ax0_copy.start()
    for j in range(6):
        for cp in qkv_copies(j):
            cp.start()

    def unpack(w, par):
        return pltpu.bitcast((w << 16) if par == 0 else (w & jnp.uint32(0xFFFF0000)), f32)

    mf_copy.wait()
    tab_copy.wait()
    row0 = lax.broadcasted_iota(jnp.int32, (8, 128), 0) == 0

    def fwd(j, carry):
        bx_copy(j).wait()
        for cp in qkv_copies(j + 6):
            cp.start()
        zs = []
        for par in range(2):
            sig = _split8([unpack(bx[j, :, t * 128:(t + 1) * 128], par) for t in range(8)])
            zs.append([_nt(mf[g], jnp.concatenate([sig[2 * g].astype(bf16), sig[2 * g + 1].astype(bf16)], axis=1))
                       for g in range(NT)])
        for par in range(2):
            z = zs[par]
            head = z[0][128:136]
            re = [zg[:128] for zg in z] + [jnp.where(row0, head, 0.0)]
            im = [jnp.where(row0, 0.0, head), z[0][136:]] + [zg[128:] for zg in z[1:]] + [jnp.zeros((8, 128), f32)]
            lhs = jnp.concatenate([jnp.concatenate(re, axis=0), jnp.concatenate(im, axis=0)], axis=1)
            n1 = 2 * j + par
            tr = jnp.tile(tab[2, pl.ds(pl.multiple_of(8 * n1, 8), 8), :], (P // 8, 1))
            ti = jnp.tile(tab[3, pl.ds(pl.multiple_of(8 * n1, 8), 8), :], (P // 8, 1))
            gr, gi = tab[0] * tr - tab[1] * ti, tab[0] * ti + tab[1] * tr
            gm = jnp.concatenate([jnp.concatenate([gr, gi], axis=1),
                                  jnp.concatenate([-gi, gr], axis=1)], axis=0).astype(bf16)
            gf[n1] = gm
            tp[n1] = jnp.dot(lhs, gm, preferred_element_type=f32)
        return carry

    lax.fori_loop(0, R // 2, fwd, 0)
    for cp in qkv_copies(14) + qkv_copies(15) + wo_copies + [ax_copy]:
        cp.start()

    for cp in w_copies:
        cp.wait()

    def filt(r0, w_of):
        xs = _fft16([(tp[n1, pl.ds(r0, 8), :P], tp[n1, pl.ds(r0, 8), P:]) for n1 in range(R)], -1)
        ys = []
        for k1, (ur, ui) in enumerate(xs):
            a, b = w_of(k1)
            ys.append((ur * a - ui * b, ur * b + ui * a))
        for n1, (yr, yi) in enumerate(_fft16(ys, 1)):
            tp[n1, pl.ds(r0, 8), :P] = yr
            tp[n1, pl.ds(r0, 8), P:] = yi

    even = lax.broadcasted_iota(jnp.int32, (8, 128), 0) % 2 == 0
    for g in range(NT):
        def body(i, carry, g=g):
            def w_of(k1):
                def rows(ref):
                    def ld(q):
                        return ref[k1, pl.ds(16 * i + q, 8, stride=2), :]
                    if g % 2 == 0:
                        return unpack(ld(g // 2), 0)
                    return unpack(jnp.where(even, ld(g // 2), ld(1 - g // 2)), 1)
                a, b = rows(wr), rows(wi)
                if g == 0:
                    half0 = jnp.where(row0 & (i == 0), 0.5, 1.0)
                    a, b = a * half0, b * half0
                return a, b
            filt(pl.multiple_of(g * 128 + 8 * i, 8), w_of)
            return carry
        lax.fori_loop(0, 16, body, 0)
    filt(D // 2, lambda k1: (jnp.where(row0, wrn_ref[:, k1 * P:(k1 + 1) * P].astype(f32), 0.0) * 0.5,
                             jnp.where(row0, win_ref[:, k1 * P:(k1 + 1) * P].astype(f32), 0.0) * 0.5))

    lane0 = lax.broadcasted_iota(jnp.int32, (P, 128), 1) == 0

    def inv(j, carry):
        ts = []
        for par in range(2):
            n1 = 2 * j + par
            ts.append([_nt(gf[n1], tp[n1, t * 128:(t + 1) * 128, :].astype(bf16)) for t in range(NT)])
        for par in range(2):
            n1 = 2 * j + par
            ny = jnp.concatenate([tp[n1, D // 2:, :], jnp.zeros((120, 2 * P), f32)], axis=0)
            ts[par].append(_nt(gf[n1, :P, :], ny.astype(bf16)))
        sig = [[], []]
        for g in range(NT):
            rows = []
            for par in range(2):
                t = ts[par][g]
                ti = jnp.where(lane0, ts[par][NT], t[P:]) if g == 0 else t[P:]
                rows.append(jnp.concatenate([t[:P], ti], axis=1))
            o = jnp.dot(jnp.concatenate(rows, axis=0), mf[g], preferred_element_type=f32)
            for par in range(2):
                sig[par] += [o[par * P:(par + 1) * P, :128], o[par * P:(par + 1) * P, 128:]]
        y0, y1 = _merge8(sig[0]), _merge8(sig[1])
        for t in range(8):
            bx[j, :, t * 128:(t + 1) * 128] = pltpu.pack_elementwise([y0[t], y1[t]], packed_dtype=bf16)
        return carry

    lax.fori_loop(0, R // 2, inv, 0)

    row = lax.broadcasted_iota(jnp.int32, (L, L), 0)
    col = lax.broadcasted_iota(jnp.int32, (L, L), 1)
    mask = (row < M) | (row >= col)
    scale = np.float32(DH ** -0.5)
    wsplit = wqkv.reshape(3 * (H // 2), D // 16, 16, 128)

    def out_copy(s):
        return pltpu.make_async_copy(oa.at[pl.ds(2 * s, 2)], out_hbm.at[pl.ds(2 * s, 2), :, pl.ds(0, D)], sem_out.at[0])

    def load_tokens(s):
        hbuf[M:L, :] = ax[pl.ds(pl.multiple_of(s * SEG, SEG), SEG), :].astype(f32)

    def proj(j, par, slot):
        for m in range(3):
            w = wsplit[m * (H // 2) + j, :, 8 * par:8 * par + 8, :].reshape(D // 2, 128)
            qkv[slot, m] = jnp.dot(hbuf[...], pltpu.bitcast(w, bf16), preferred_element_type=f32)

    def scores(slot):
        sc = _nt(qkv[slot, 0], qkv[slot, 1]) * scale
        sc = jnp.where(mask, sc, -1e9)
        e = jnp.exp(sc - jnp.max(sc, axis=-1, keepdims=True))
        pbuf[slot % 4] = e / jnp.sum(e, axis=-1, keepdims=True)

    def pv(h, slot):
        obuf[h] = jnp.dot(pbuf[slot % 4], qkv[slot, 2], preferred_element_type=f32)

    def oproj(c, h0, h1):
        o = jnp.concatenate([obuf[h] for h in range(h0, h1)], axis=1)
        return jnp.dot(o, pltpu.bitcast(wo[c, 64 * h0:64 * h1, :], bf16), preferred_element_type=f32)

    def finish(s, c, o):
        hbuf[0:M, 128 * c:128 * (c + 1)] = o[0:M].astype(bf16).astype(f32)
        oa[pl.ds(2 * s, 2), :, 128 * c:128 * (c + 1)] = o[M:L].astype(bf16).reshape(2, R, 128)

    mem_copy.wait()
    ax0_copy.wait()
    hbuf[0:M, :] = mem_ref[...].astype(f32)
    load_tokens(0)

    def first(j, carry):
        for cp in qkv_copies(j):
            cp.wait()

        def split(g, carry):
            jj = (g // 4) * (H // 2) + j
            base = pl.multiple_of((g % 4) * 256, 256)
            ev = [wqkv[jj, pl.ds(base + 16 * i, 8, stride=2), :] for i in range(16)]
            od = [wqkv[jj, pl.ds(base + 16 * i + 1, 8, stride=2), :] for i in range(16)]
            for i in range(16):
                wqkv[jj, pl.ds(base + 16 * i, 8), :] = (ev[i] & 0xFFFF) | (od[i] << 16)
                wqkv[jj, pl.ds(base + 16 * i + 8, 8), :] = (ev[i] >> 16) | (od[i] & jnp.uint32(0xFFFF0000))
            return carry

        lax.fori_loop(0, 12, split, 0)
        for par in range(2):
            proj(j, par, par)
        for par in range(2):
            scores(par)
        for par in range(2):
            pv(2 * j + par, par)
        return carry

    lax.fori_loop(0, H // 2, first, 0)
    for c in range(D // 128):
        wo_copies[c].wait()
        finish(0, c, oproj(c, 0, H))
    out_copy(0).start()
    for j in range(R // 2):
        y_copy(j).start()
    ax_copy.wait()

    def seg(s, carry):
        load_tokens(s)
        for g in range(H // 4):
            prev = range(4 * g - 4, 4 * g) if g else ()
            proj(2 * g, 0, (4 * g) % 8)
            for h in prev:
                scores(h % 8)
            for h in range(4 * g + 1, 4 * g + 4):
                proj(h // 2, h % 2, h % 8)
            for h in prev:
                pv(h, h % 8)
        part[0] = oproj(0, 0, 24)
        for h in range(H - 4, H):
            scores(h % 8)
        part[1] = oproj(1, 0, 28)
        part[2] = oproj(2, 0, 28)
        for h in range(H - 4, H):
            pv(h, h % 8)
        part[3] = oproj(3, 0, 28)
        finish(s, 0, part[0] + oproj(0, 24, 32))
        for c in range(1, 4):
            finish(s, c, part[c] + oproj(c, 28, 32))
        for c in range(4, 8):
            finish(s, c, oproj(c, 0, 32))
        out_copy(s).start()
        return carry

    lax.fori_loop(1, NSEG, seg, 0, unroll=3)

    def drain(s, carry):
        out_copy(s).wait()
        return carry

    lax.fori_loop(0, NSEG, drain, 0)
    for j in range(R // 2):
        y_copy(j).wait()


@functools.partial(jax.jit, static_argnames=("A_seg_len",))
def pallas_concat_heads__memory_aug_recurrent_mem_tr__spectral_gfnet__prompt_kernel(
    A_x, A_mem0, A_Wq, A_Wk, A_Wv, A_Wo, A_seg_len, B_x, B_w_r, B_w_i,
):
    assert A_seg_len == SEG and A_x.shape == (1, S, D) and B_x.shape == (1, S, D)
    mf, tab = _constants()
    hbm = pl.BlockSpec(memory_space=pltpu.HBM)
    nyq = pl.BlockSpec((8, S), lambda i: (D // 16, 0))
    wr, wi = B_w_r.T, B_w_i.T
    out = pl.pallas_call(
        _kernel,
        out_shape=jax.ShapeDtypeStruct((P, R, 2 * D), bf16),
        grid=(1,),
        in_specs=[hbm] * 9 + [nyq, nyq] + [hbm] * 2,
        out_specs=hbm,
        scratch_shapes=[
            pltpu.VMEM((3 * H // 2, D, 128), u32),
            pltpu.VMEM((D // 128, H * DH // 2, 128), u32),
            pltpu.VMEM((S, D), bf16),
            pltpu.VMEM((P, R, D), bf16),
            pltpu.VMEM((R // 2, P, D), u32),
            pltpu.VMEM((NT, 256, 256), bf16),
            pltpu.VMEM((4, P, P), f32),
            pltpu.VMEM((R, 2 * P, 2 * P), bf16),
            pltpu.VMEM((R, D // 4, P), u32),
            pltpu.VMEM((R, D // 4, P), u32),
            pltpu.VMEM((R, D // 2 + 8, 2 * P), f32),
            pltpu.VMEM((M, D), bf16),
            pltpu.VMEM((L, D), f32),
            pltpu.VMEM((H, L, DH), f32),
            pltpu.VMEM((8, 3, L, DH), f32),
            pltpu.VMEM((4, L, L), f32),
            pltpu.VMEM((4, L, 128), f32),
            pltpu.SemaphoreType.DMA((R // 2,)),
            pltpu.SemaphoreType.DMA((H // 2,)),
            pltpu.SemaphoreType.DMA((D // 128,)),
            pltpu.SemaphoreType.DMA((12,)),
            pltpu.SemaphoreType.DMA((1,)),
        ],
        compiler_params=pltpu.CompilerParams(vmem_limit_bytes=110 * 2**20),
        name="rmt_gfnet",
    )(A_x.reshape(S, D), A_mem0.reshape(M, D), A_Wq, A_Wk, A_Wv, A_Wo.reshape(H * DH, D),
      B_x.reshape(P, R, D), wr, wi, wr, wi, mf, tab)
    return out.reshape(1, S, 2 * D)
```

```python
import functools

import jax
import jax.numpy as jnp
import numpy as np
from jax import lax
import jax.experimental.pallas as pl
import jax.experimental.pallas.tpu as pltpu

f32, bf16, u32 = jnp.float32, jnp.bfloat16, jnp.uint32

S, D = 2048, 1024
H, DH, M, SEG = 32, 128, 8, 32
L = M + SEG
NSEG = S // SEG
UNROLL = 3
NTRIP = (NSEG - 1) // UNROLL
R, P = 16, 128
NT = D // 2 // 128


_RT = float(np.sqrt(0.5))


def _split8(x):
    a0, a1, b0, b1 = x[0] + x[4], x[0] - x[4], x[2] + x[6], x[2] - x[6]
    c0, c1, d0, d1 = x[1] + x[5], x[1] - x[5], x[3] + x[7], x[3] - x[7]
    e, f = a0 + b0, c0 + d0
    u, v = (c1 - d1) * _RT, (c1 + d1) * _RT
    return [e + f, e - f, a1 + u, b1 + v, a0 - b0, c0 - d0, a1 - u, b1 - v]


def _merge8(y):
    e, f = y[0] + y[1], y[0] - y[1]
    a0, b0, c0, d0 = e + y[4], e - y[4], f + y[5], f - y[5]
    a1, b1 = y[2] + y[6], y[3] + y[7]
    u, v = (y[2] - y[6]) * _RT, (y[3] - y[7]) * _RT
    c1, d1 = u + v, v - u
    return [a0 + a1, c0 + c1, b0 + b1, d0 + d1, a0 - a1, c0 - c1, b0 - b1, d0 - d1]


_GROUPS = ((0, 4), (1, 7), (2, 6), (3, 5))


@functools.lru_cache(maxsize=None)
def _constants():
    basis = np.stack(_split8(list(np.eye(8))))
    d = np.arange(D)[None, :]
    mf = []
    for g, ks in enumerate(_GROUPS):
        kd = np.sort(np.concatenate([k1 + 8 * np.arange(64) for k1 in ks]))[:, None]
        ang = 2.0 * np.pi * ((d * kd) % D) / D
        rows = np.concatenate([np.cos(ang), -np.sin(ang)], axis=0)
        if g == 0:
            rows[128] = 1.0 - 2.0 * (np.arange(D) % 2)
        bg = basis[2 * g:2 * g + 2]
        rows = rows.reshape(256, 8, 128)
        m = np.einsum("oad,as->osd", rows, np.linalg.pinv(bg))
        assert np.abs(np.einsum("osd,sa->oad", m, bg) - rows).max() < 1e-9
        mf.append(m.reshape(256, 256))
    k2 = np.arange(P)[None, :]
    a = 2.0 * np.pi * ((np.arange(P)[:, None] * k2) % P) / P
    t = 2.0 * np.pi * (np.repeat(np.arange(R), 8)[:, None] * k2) / S
    tab = np.stack([np.cos(a), -np.sin(a), np.cos(t) * 2.0 ** -10, -np.sin(t) * 2.0 ** -10])
    return np.stack(mf).astype(bf16), tab.astype(np.float32)


def _fft16(xs, sign):
    def bf4(a, b, c, d):
        s0 = (a[0] + c[0], a[1] + c[1])
        s1 = (a[0] - c[0], a[1] - c[1])
        s2 = (b[0] + d[0], b[1] + d[1])
        s3 = (b[0] - d[0], b[1] - d[1])
        p = (s1[0] - s3[1], s1[1] + s3[0])
        m = (s1[0] + s3[1], s1[1] - s3[0])
        o1, o3 = (p, m) if sign > 0 else (m, p)
        return [(s0[0] + s2[0], s0[1] + s2[1]), o1, (s0[0] - s2[0], s0[1] - s2[1]), o3]

    def tw(x, e):
        e = e % 16
        if e == 0:
            return x
        if e == 4:
            return (-x[1], x[0]) if sign > 0 else (x[1], -x[0])
        c = np.float32(np.cos(2 * np.pi * e / 16))
        s = np.float32(sign * np.sin(2 * np.pi * e / 16))
        if e == 2:
            return ((x[0] - x[1]) * c, (x[0] + x[1]) * c) if sign > 0 else ((x[0] + x[1]) * c, (x[1] - x[0]) * c)
        if e == 6:
            return ((x[0] + x[1]) * c, (x[1] - x[0]) * c) if sign > 0 else ((x[0] - x[1]) * c, (x[0] + x[1]) * c)
        return (x[0] * c - x[1] * s, x[0] * s + x[1] * c)

    inner = [bf4(xs[b], xs[4 + b], xs[8 + b], xs[12 + b]) for b in range(4)]
    out = [None] * 16
    for c in range(4):
        o = bf4(*[tw(inner[b][c], b * c) for b in range(4)])
        for e in range(4):
            out[c + 4 * e] = o[e]
    return out


def _nt(a, b):
    return lax.dot_general(a, b, (((1,), (1,)), ((), ())), preferred_element_type=f32)


def _kernel(ax_hbm, mem_hbm, wq_hbm, wk_hbm, wv_hbm, wo_hbm, bx_hbm, wr_hbm, wi_hbm, wrn_ref, win_ref,
            mf_hbm, tab_hbm, out_hbm,
            wqkv, wo, ax, oa, bx, mf, tab, gf, wr, wi, tp, mem_ref,
            hbuf, obuf, qkv, pbuf, part, sem_bx, sem_qkv, sem_wo, sem, sem_out):
    bx32 = bx_hbm.bitcast(u32)
    out32 = out_hbm.bitcast(u32)

    def bx_copy(j):
        return pltpu.make_async_copy(bx32.at[:, j, :], bx.at[j], sem_bx.at[j])

    def y_copy(j):
        return pltpu.make_async_copy(bx.at[j], out32.at[:, j, pl.ds(D, D)], sem.at[10])

    mf_copy = pltpu.make_async_copy(mf_hbm, mf, sem.at[0])
    tab_copy = pltpu.make_async_copy(tab_hbm, tab, sem.at[1])

    ax0_copy = pltpu.make_async_copy(ax_hbm.at[pl.ds(0, SEG), :], ax.at[1, pl.ds(0, SEG), :], sem.at[2])

    def ax_copy(t):
        r0 = pl.multiple_of(SEG + jnp.minimum(t, NTRIP - 1) * (UNROLL * SEG), SEG)
        return pltpu.make_async_copy(ax_hbm.at[pl.ds(r0, UNROLL * SEG), :], ax.at[t % 2], sem.at[2])

    mem_copy = pltpu.make_async_copy(mem_hbm, mem_ref, sem.at[11])
    w_copies = [pltpu.make_async_copy(src.at[pl.ds(0, D // 2), pl.ds(k1 * P, P)].bitcast(u32), dst.at[k1], sem.at[5])
                for src, dst in ((wr_hbm, wr), (wi_hbm, wi)) for k1 in range(R)]

    def qkv_copies(j):
        return [pltpu.make_async_copy(src.bitcast(u32).at[:, j, :], wqkv.at[m * (H // 2) + j], sem_qkv.at[j])
                for m, src in enumerate((wq_hbm, wk_hbm, wv_hbm))]

    wo32 = wo_hbm.bitcast(u32)
    wo_copies = [pltpu.make_async_copy(wo32.at[:, pl.ds(c * 128, 128)], wo.at[c], sem_wo.at[c]) for c in range(D // 128)]

    mf_copy.start()
    bx_copy(0).start()
    tab_copy.start()
    for j in range(1, R // 2):
        bx_copy(j).start()
    for cp in w_copies:
        cp.start()
    mem_copy.start()
    ax0_copy.start()

    def unpack(w, par):
        return pltpu.bitcast((w << 16) if par == 0 else (w & jnp.uint32(0xFFFF0000)), f32)

    mf_copy.wait()
    tab_copy.wait()
    row0 = lax.broadcasted_iota(jnp.int32, (8, 128), 0) == 0

    def fwd(j, carry):
        bx_copy(j).wait()

        @pl.when(j == 5)
        def _():
            for jj in range(H // 2):
                for cp in qkv_copies(jj):
                    cp.start()

        zs = []
        for par in range(2):
            sig = _split8([unpack(bx[j, :, t * 128:(t + 1) * 128], par) for t in range(8)])
            zs.append([_nt(mf[g], jnp.concatenate([sig[2 * g].astype(bf16), sig[2 * g + 1].astype(bf16)], axis=1))
                       for g in range(NT)])
        for par in range(2):
            z = zs[par]
            head = z[0][128:136]
            re = [zg[:128] for zg in z] + [jnp.where(row0, head, 0.0)]
            im = [jnp.where(row0, 0.0, head), z[0][136:]] + [zg[128:] for zg in z[1:]] + [jnp.zeros((8, 128), f32)]
            lhs = jnp.concatenate([jnp.concatenate(re, axis=0), jnp.concatenate(im, axis=0)], axis=1)
            n1 = 2 * j + par
            tr = jnp.tile(tab[2, pl.ds(pl.multiple_of(8 * n1, 8), 8), :], (P // 8, 1))
            ti = jnp.tile(tab[3, pl.ds(pl.multiple_of(8 * n1, 8), 8), :], (P // 8, 1))
            gr, gi = tab[0] * tr - tab[1] * ti, tab[0] * ti + tab[1] * tr
            gm = jnp.concatenate([jnp.concatenate([gr, gi], axis=1),
                                  jnp.concatenate([-gi, gr], axis=1)], axis=0).astype(bf16)
            gf[n1] = gm
            tp[n1] = jnp.dot(lhs, gm, preferred_element_type=f32)
        return carry

    lax.fori_loop(0, R // 2, fwd, 0)

    for cp in w_copies:
        cp.wait()

    def filt(r0, w_of):
        xs = _fft16([(tp[n1, pl.ds(r0, 8), :P], tp[n1, pl.ds(r0, 8), P:]) for n1 in range(R)], -1)
        ys = []
        for k1, (ur, ui) in enumerate(xs):
            a, b = w_of(k1)
            ys.append((ur * a - ui * b, ur * b + ui * a))
        for n1, (yr, yi) in enumerate(_fft16(ys, 1)):
            tp[n1, pl.ds(r0, 8), :P] = yr
            tp[n1, pl.ds(r0, 8), P:] = yi

    even = lax.broadcasted_iota(jnp.int32, (8, 128), 0) % 2 == 0
    for g in range(NT):
        def body(i, carry, g=g):
            def w_of(k1):
                def rows(ref):
                    def ld(q):
                        return ref[k1, pl.ds(16 * i + q, 8, stride=2), :]
                    if g % 2 == 0:
                        return unpack(ld(g // 2), 0)
                    return unpack(jnp.where(even, ld(g // 2), ld(1 - g // 2)), 1)
                a, b = rows(wr), rows(wi)
                if g == 0:
                    half0 = jnp.where(row0 & (i == 0), 0.5, 1.0)
                    a, b = a * half0, b * half0
                return a, b
            filt(pl.multiple_of(g * 128 + 8 * i, 8), w_of)
            return carry
        lax.fori_loop(0, 16, body, 0)
    filt(D // 2, lambda k1: (jnp.where(row0, wrn_ref[:, k1 * P:(k1 + 1) * P].astype(f32), 0.0) * 0.5,
                             jnp.where(row0, win_ref[:, k1 * P:(k1 + 1) * P].astype(f32), 0.0) * 0.5))

    for cp in wo_copies:
        cp.start()
    lane0 = lax.broadcasted_iota(jnp.int32, (P, 128), 1) == 0

    def inv(j, carry):
        ts = []
        for par in range(2):
            n1 = 2 * j + par
            ts.append([_nt(gf[n1], tp[n1, t * 128:(t + 1) * 128, :].astype(bf16)) for t in range(NT)])
        for par in range(2):
            n1 = 2 * j + par
            ny = jnp.concatenate([tp[n1, D // 2:, :], jnp.zeros((120, 2 * P), f32)], axis=0)
            ts[par].append(_nt(gf[n1, :P, :], ny.astype(bf16)))
        sig = [[], []]
        for g in range(NT):
            rows = []
            for par in range(2):
                t = ts[par][g]
                ti = jnp.where(lane0, ts[par][NT], t[P:]) if g == 0 else t[P:]
                rows.append(jnp.concatenate([t[:P], ti], axis=1))
            o = jnp.dot(jnp.concatenate(rows, axis=0), mf[g], preferred_element_type=f32)
            for par in range(2):
                sig[par] += [o[par * P:(par + 1) * P, :128], o[par * P:(par + 1) * P, 128:]]
        y0, y1 = _merge8(sig[0]), _merge8(sig[1])
        for t in range(8):
            bx[j, :, t * 128:(t + 1) * 128] = pltpu.pack_elementwise([y0[t], y1[t]], packed_dtype=bf16)
        return carry

    lax.fori_loop(0, R // 2, inv, 0)

    row = lax.broadcasted_iota(jnp.int32, (L, L), 0)
    col = lax.broadcasted_iota(jnp.int32, (L, L), 1)
    mask = (row < M) | (row >= col)
    scale = np.float32(DH ** -0.5)
    wsplit = wqkv.reshape(3 * (H // 2), D // 16, 16, 128)

    def out_copy(s):
        return pltpu.make_async_copy(oa.at[pl.ds(2 * s, 2)], out_hbm.at[pl.ds(2 * s, 2), :, pl.ds(0, D)], sem_out.at[0])

    def load_tokens(slot, u):
        hbuf[M:L, :] = ax[slot, u * SEG:(u + 1) * SEG, :].astype(f32)

    def proj(j, par, slot):
        for m in range(3):
            w = wsplit[m * (H // 2) + j, :, 8 * par:8 * par + 8, :].reshape(D // 2, 128)
            qkv[slot, m] = jnp.dot(hbuf[...], pltpu.bitcast(w, bf16), preferred_element_type=f32)

    def scores(slot):
        sc = _nt(qkv[slot, 0], qkv[slot, 1]) * scale
        sc = jnp.where(mask, sc, -1e9)
        e = jnp.exp(sc - jnp.max(sc, axis=-1, keepdims=True))
        pbuf[slot % 4] = e / jnp.sum(e, axis=-1, keepdims=True)

    def pv(h, slot):
        obuf[h] = jnp.dot(pbuf[slot % 4], qkv[slot, 2], preferred_element_type=f32)

    def oproj(c, h0, h1):
        o = jnp.concatenate([obuf[h] for h in range(h0, h1)], axis=1)
        return jnp.dot(o, pltpu.bitcast(wo[c, 64 * h0:64 * h1, :], bf16), preferred_element_type=f32)

    def finish(s, c, o):
        hbuf[0:M, 128 * c:128 * (c + 1)] = o[0:M].astype(bf16).astype(f32)
        oa[pl.ds(2 * s, 2), :, 128 * c:128 * (c + 1)] = o[M:L].astype(bf16).reshape(2, R, 128)

    mem_copy.wait()
    ax0_copy.wait()
    ax_copy(0).start()
    hbuf[0:M, :] = mem_ref[...].astype(f32)
    load_tokens(1, 0)

    def first(j, carry):
        for cp in qkv_copies(j):
            cp.wait()

        def split(g, carry):
            jj = (g // 4) * (H // 2) + j
            base = pl.multiple_of((g % 4) * 256, 256)
            ev = [wqkv[jj, pl.ds(base + 16 * i, 8, stride=2), :] for i in range(16)]
            od = [wqkv[jj, pl.ds(base + 16 * i + 1, 8, stride=2), :] for i in range(16)]
            for i in range(16):
                wqkv[jj, pl.ds(base + 16 * i, 8), :] = (ev[i] & 0xFFFF) | (od[i] << 16)
                wqkv[jj, pl.ds(base + 16 * i + 8, 8), :] = (ev[i] >> 16) | (od[i] & jnp.uint32(0xFFFF0000))
            return carry

        lax.fori_loop(0, 12, split, 0)
        for par in range(2):
            proj(j, par, par)
        for par in range(2):
            scores(par)
        for par in range(2):
            pv(2 * j + par, par)
        return carry

    lax.fori_loop(0, H // 2, first, 0)
    for c in range(D // 128):
        wo_copies[c].wait()
        finish(0, c, oproj(c, 0, H))
    out_copy(0).start()
    for j in range(R // 2):
        y_copy(j).start()

    def seg(s):
        for g in range(H // 4):
            prev = range(4 * g - 4, 4 * g) if g else ()
            proj(2 * g, 0, (4 * g) % 8)
            for h in prev:
                scores(h % 8)
            for h in range(4 * g + 1, 4 * g + 4):
                proj(h // 2, h % 2, h % 8)
            for h in prev:
                pv(h, h % 8)
        part[0] = oproj(0, 0, 24)
        for h in range(H - 4, H):
            scores(h % 8)
        part[1] = oproj(1, 0, 28)
        part[2] = oproj(2, 0, 28)
        for h in range(H - 4, H):
            pv(h, h % 8)
        part[3] = oproj(3, 0, 28)
        finish(s, 0, part[0] + oproj(0, 24, 32))
        for c in range(1, 4):
            finish(s, c, part[c] + oproj(c, 28, 32))
        for c in range(4, 8):
            finish(s, c, oproj(c, 0, 32))

    def trip(t, carry):
        ax_copy(t).wait()
        ax_copy(t + 1).start()
        for u in range(UNROLL):
            load_tokens(t % 2, u)
            seg(1 + UNROLL * t + u)
        for u in range(UNROLL):
            out_copy(1 + UNROLL * t + u).start()
        return carry

    lax.fori_loop(0, NTRIP, trip, 0)
    ax_copy(NTRIP).wait()

    def drain(s, carry):
        out_copy(s).wait()
        return carry

    lax.fori_loop(0, NSEG, drain, 0)
    for j in range(R // 2):
        y_copy(j).wait()


@functools.partial(jax.jit, static_argnames=("A_seg_len",))
def pallas_concat_heads__memory_aug_recurrent_mem_tr__spectral_gfnet__prompt_kernel(
    A_x, A_mem0, A_Wq, A_Wk, A_Wv, A_Wo, A_seg_len, B_x, B_w_r, B_w_i,
):
    assert A_seg_len == SEG and A_x.shape == (1, S, D) and B_x.shape == (1, S, D)
    mf, tab = _constants()
    hbm = pl.BlockSpec(memory_space=pltpu.HBM)
    nyq = pl.BlockSpec((8, S), lambda i: (D // 16, 0))
    wr, wi = B_w_r.T, B_w_i.T
    out = pl.pallas_call(
        _kernel,
        out_shape=jax.ShapeDtypeStruct((P, R, 2 * D), bf16),
        grid=(1,),
        in_specs=[hbm] * 9 + [nyq, nyq] + [hbm] * 2,
        out_specs=hbm,
        scratch_shapes=[
            pltpu.VMEM((3 * H // 2, D, 128), u32),
            pltpu.VMEM((D // 128, H * DH // 2, 128), u32),
            pltpu.VMEM((2, UNROLL * SEG, D), bf16),
            pltpu.VMEM((P, R, D), bf16),
            pltpu.VMEM((R // 2, P, D), u32),
            pltpu.VMEM((NT, 256, 256), bf16),
            pltpu.VMEM((4, P, P), f32),
            pltpu.VMEM((R, 2 * P, 2 * P), bf16),
            pltpu.VMEM((R, D // 4, P), u32),
            pltpu.VMEM((R, D // 4, P), u32),
            pltpu.VMEM((R, D // 2 + 8, 2 * P), f32),
            pltpu.VMEM((M, D), bf16),
            pltpu.VMEM((L, D), f32),
            pltpu.VMEM((H, L, DH), f32),
            pltpu.VMEM((8, 3, L, DH), f32),
            pltpu.VMEM((4, L, L), f32),
            pltpu.VMEM((4, L, 128), f32),
            pltpu.SemaphoreType.DMA((R // 2,)),
            pltpu.SemaphoreType.DMA((H // 2,)),
            pltpu.SemaphoreType.DMA((D // 128,)),
            pltpu.SemaphoreType.DMA((12,)),
            pltpu.SemaphoreType.DMA((1,)),
        ],
        compiler_params=pltpu.CompilerParams(vmem_limit_bytes=110 * 2**20),
        name="rmt_gfnet",
    )(A_x.reshape(S, D), A_mem0.reshape(M, D), A_Wq, A_Wk, A_Wv, A_Wo.reshape(H * DH, D),
      B_x.reshape(P, R, D), wr, wi, wr, wi, mf, tab)
    return out.reshape(1, S, 2 * D)
```

```python
import functools

import jax
import jax.numpy as jnp
import numpy as np
from jax import lax
import jax.experimental.pallas as pl
import jax.experimental.pallas.tpu as pltpu

f32, bf16, u32 = jnp.float32, jnp.bfloat16, jnp.uint32

S, D = 2048, 1024
H, DH, M, SEG = 32, 128, 8, 32
L = M + SEG
NSEG = S // SEG
UNROLL = 3
NTRIP = (NSEG - 1) // UNROLL
R, P = 16, 128
NT = D // 2 // 128


_RT = float(np.sqrt(0.5))


def _split8(x):
    a0, a1, b0, b1 = x[0] + x[4], x[0] - x[4], x[2] + x[6], x[2] - x[6]
    c0, c1, d0, d1 = x[1] + x[5], x[1] - x[5], x[3] + x[7], x[3] - x[7]
    e, f = a0 + b0, c0 + d0
    u, v = (c1 - d1) * _RT, (c1 + d1) * _RT
    return [e + f, e - f, a1 + u, b1 + v, a0 - b0, c0 - d0, a1 - u, b1 - v]


def _merge8(y):
    e, f = y[0] + y[1], y[0] - y[1]
    a0, b0, c0, d0 = e + y[4], e - y[4], f + y[5], f - y[5]
    a1, b1 = y[2] + y[6], y[3] + y[7]
    u, v = (y[2] - y[6]) * _RT, (y[3] - y[7]) * _RT
    c1, d1 = u + v, v - u
    return [a0 + a1, c0 + c1, b0 + b1, d0 + d1, a0 - a1, c0 - c1, b0 - b1, d0 - d1]


_GROUPS = ((0, 4), (1, 7), (2, 6), (3, 5))


@functools.lru_cache(maxsize=None)
def _constants():
    basis = np.stack(_split8(list(np.eye(8))))
    d = np.arange(D)[None, :]
    mf = []
    for g, ks in enumerate(_GROUPS):
        kd = np.sort(np.concatenate([k1 + 8 * np.arange(64) for k1 in ks]))[:, None]
        ang = 2.0 * np.pi * ((d * kd) % D) / D
        rows = np.concatenate([np.cos(ang), -np.sin(ang)], axis=0)
        if g == 0:
            rows[128] = 1.0 - 2.0 * (np.arange(D) % 2)
        bg = basis[2 * g:2 * g + 2]
        rows = rows.reshape(256, 8, 128)
        m = np.einsum("oad,as->osd", rows, np.linalg.pinv(bg))
        assert np.abs(np.einsum("osd,sa->oad", m, bg) - rows).max() < 1e-9
        mf.append(m.reshape(256, 256))
    k2 = np.arange(P)[None, :]
    a = 2.0 * np.pi * ((np.arange(P)[:, None] * k2) % P) / P
    t = 2.0 * np.pi * (np.repeat(np.arange(R), 8)[:, None] * k2) / S
    tab = np.stack([np.cos(a), -np.sin(a), np.cos(t) * 2.0 ** -10, -np.sin(t) * 2.0 ** -10])
    return np.stack(mf).astype(bf16), tab.astype(np.float32)


def _fft16(xs, sign):
    def bf4(a, b, c, d):
        s0 = (a[0] + c[0], a[1] + c[1])
        s1 = (a[0] - c[0], a[1] - c[1])
        s2 = (b[0] + d[0], b[1] + d[1])
        s3 = (b[0] - d[0], b[1] - d[1])
        p = (s1[0] - s3[1], s1[1] + s3[0])
        m = (s1[0] + s3[1], s1[1] - s3[0])
        o1, o3 = (p, m) if sign > 0 else (m, p)
        return [(s0[0] + s2[0], s0[1] + s2[1]), o1, (s0[0] - s2[0], s0[1] - s2[1]), o3]

    def tw(x, e):
        e = e % 16
        if e == 0:
            return x
        if e == 4:
            return (-x[1], x[0]) if sign > 0 else (x[1], -x[0])
        c = np.float32(np.cos(2 * np.pi * e / 16))
        s = np.float32(sign * np.sin(2 * np.pi * e / 16))
        if e == 2:
            return ((x[0] - x[1]) * c, (x[0] + x[1]) * c) if sign > 0 else ((x[0] + x[1]) * c, (x[1] - x[0]) * c)
        if e == 6:
            return ((x[0] + x[1]) * c, (x[1] - x[0]) * c) if sign > 0 else ((x[0] - x[1]) * c, (x[0] + x[1]) * c)
        return (x[0] * c - x[1] * s, x[0] * s + x[1] * c)

    inner = [bf4(xs[b], xs[4 + b], xs[8 + b], xs[12 + b]) for b in range(4)]
    out = [None] * 16
    for c in range(4):
        o = bf4(*[tw(inner[b][c], b * c) for b in range(4)])
        for e in range(4):
            out[c + 4 * e] = o[e]
    return out


def _nt(a, b):
    return lax.dot_general(a, b, (((1,), (1,)), ((), ())), preferred_element_type=f32)


def _kernel(ax_hbm, mem_hbm, wq_hbm, wk_hbm, wv_hbm, wo_hbm, bx_hbm, wr_hbm, wi_hbm, wrn_ref, win_ref,
            mf_hbm, tab_hbm, out_hbm,
            wqkv, wo, ax, oa, bx, mf, tab, gf, wr, wi, tp, mem_ref,
            hbuf, obuf, qkv, pbuf, part, sem_bx, sem_qkv, sem_wo, sem, sem_out):
    bx32 = bx_hbm.bitcast(u32)
    out32 = out_hbm.bitcast(u32)

    def bx_copy(j):
        return pltpu.make_async_copy(bx32.at[:, j, :], bx.at[j], sem_bx.at[j])

    def y_copy(j):
        return pltpu.make_async_copy(bx.at[j], out32.at[:, j, pl.ds(D, D)], sem.at[10])

    mf_copy = pltpu.make_async_copy(mf_hbm, mf, sem.at[0])
    tab_copy = pltpu.make_async_copy(tab_hbm, tab, sem.at[1])

    ax0_copy = pltpu.make_async_copy(ax_hbm.at[pl.ds(0, SEG), :], ax.at[1, pl.ds(0, SEG), :], sem.at[2])

    def ax_copy(t):
        r0 = pl.multiple_of(SEG + jnp.minimum(t, NTRIP - 1) * (UNROLL * SEG), SEG)
        return pltpu.make_async_copy(ax_hbm.at[pl.ds(r0, UNROLL * SEG), :], ax.at[t % 2], sem.at[2])

    mem_copy = pltpu.make_async_copy(mem_hbm, mem_ref, sem.at[11])
    w_copies = [pltpu.make_async_copy(src.at[pl.ds(0, D // 2), pl.ds(k1 * P, P)].bitcast(u32), dst.at[k1], sem.at[5])
                for src, dst in ((wr_hbm, wr), (wi_hbm, wi)) for k1 in range(R)]

    def qkv_copies(j):
        return [pltpu.make_async_copy(src.bitcast(u32).at[:, j, :], wqkv.at[m * (H // 2) + j], sem_qkv.at[j])
                for m, src in enumerate((wq_hbm, wk_hbm, wv_hbm))]

    wo32 = wo_hbm.bitcast(u32)
    wo_copies = [pltpu.make_async_copy(wo32.at[:, pl.ds(c * 128, 128)], wo.at[c], sem_wo.at[c]) for c in range(D // 128)]

    mf_copy.start()
    bx_copy(0).start()
    tab_copy.start()
    for j in range(1, R // 2):
        bx_copy(j).start()
    for cp in w_copies:
        cp.start()
    mem_copy.start()
    ax0_copy.start()

    def unpack(w, par):
        return pltpu.bitcast((w << 16) if par == 0 else (w & jnp.uint32(0xFFFF0000)), f32)

    mf_copy.wait()
    tab_copy.wait()
    row0 = lax.broadcasted_iota(jnp.int32, (8, 128), 0) == 0

    def fwd(j, carry):
        bx_copy(j).wait()

        @pl.when(j == 5)
        def _():
            for jj in range(H // 2):
                for cp in qkv_copies(jj):
                    cp.start()

        zs = []
        for par in range(2):
            sig = _split8([unpack(bx[j, :, t * 128:(t + 1) * 128], par) for t in range(8)])
            zs.append([_nt(mf[g], jnp.concatenate([sig[2 * g].astype(bf16), sig[2 * g + 1].astype(bf16)], axis=1))
                       for g in range(NT)])
        for par in range(2):
            z = zs[par]
            head = z[0][128:136]
            re = [zg[:128] for zg in z] + [jnp.where(row0, head, 0.0)]
            im = [jnp.where(row0, 0.0, head), z[0][136:]] + [zg[128:] for zg in z[1:]] + [jnp.zeros((8, 128), f32)]
            lhs = jnp.concatenate([jnp.concatenate(re, axis=0), jnp.concatenate(im, axis=0)], axis=1)
            n1 = 2 * j + par
            tr = jnp.tile(tab[2, pl.ds(pl.multiple_of(8 * n1, 8), 8), :], (P // 8, 1))
            ti = jnp.tile(tab[3, pl.ds(pl.multiple_of(8 * n1, 8), 8), :], (P // 8, 1))
            gr, gi = tab[0] * tr - tab[1] * ti, tab[0] * ti + tab[1] * tr
            gm = jnp.concatenate([jnp.concatenate([gr, gi], axis=1),
                                  jnp.concatenate([-gi, gr], axis=1)], axis=0).astype(bf16)
            gf[n1] = gm
            tp[n1] = jnp.dot(lhs, gm, preferred_element_type=f32)
        return carry

    lax.fori_loop(0, R // 2, fwd, 0)

    for cp in w_copies:
        cp.wait()

    def filt(r0, w_of):
        xs = _fft16([(tp[n1, pl.ds(r0, 8), :P], tp[n1, pl.ds(r0, 8), P:]) for n1 in range(R)], -1)
        ys = []
        for k1, (ur, ui) in enumerate(xs):
            a, b = w_of(k1)
            ys.append((ur * a - ui * b, ur * b + ui * a))
        for n1, (yr, yi) in enumerate(_fft16(ys, 1)):
            tp[n1, pl.ds(r0, 8), :P] = yr
            tp[n1, pl.ds(r0, 8), P:] = yi

    even = lax.broadcasted_iota(jnp.int32, (8, 128), 0) % 2 == 0
    for g in range(NT):
        def body(i, carry, g=g):
            def w_of(k1):
                def rows(ref):
                    def ld(q):
                        return ref[k1, pl.ds(16 * i + q, 8, stride=2), :]
                    if g % 2 == 0:
                        return unpack(ld(g // 2), 0)
                    return unpack(jnp.where(even, ld(g // 2), ld(1 - g // 2)), 1)
                a, b = rows(wr), rows(wi)
                if g == 0:
                    half0 = jnp.where(row0 & (i == 0), 0.5, 1.0)
                    a, b = a * half0, b * half0
                return a, b
            filt(pl.multiple_of(g * 128 + 8 * i, 8), w_of)
            return carry
        lax.fori_loop(0, 16, body, 0)
    filt(D // 2, lambda k1: (jnp.where(row0, wrn_ref[:, k1 * P:(k1 + 1) * P].astype(f32), 0.0) * 0.5,
                             jnp.where(row0, win_ref[:, k1 * P:(k1 + 1) * P].astype(f32), 0.0) * 0.5))

    for cp in wo_copies:
        cp.start()
    lane0 = lax.broadcasted_iota(jnp.int32, (P, 128), 1) == 0

    def inv(j, carry):
        ts = []
        for par in range(2):
            n1 = 2 * j + par
            ts.append([_nt(gf[n1], tp[n1, t * 128:(t + 1) * 128, :].astype(bf16)) for t in range(NT)])
        for par in range(2):
            n1 = 2 * j + par
            ny = jnp.concatenate([tp[n1, D // 2:, :], jnp.zeros((120, 2 * P), f32)], axis=0)
            ts[par].append(_nt(gf[n1, :P, :], ny.astype(bf16)))
        sig = [[], []]
        for g in range(NT):
            rows = []
            for par in range(2):
                t = ts[par][g]
                ti = jnp.where(lane0, ts[par][NT], t[P:]) if g == 0 else t[P:]
                rows.append(jnp.concatenate([t[:P], ti], axis=1))
            o = jnp.dot(jnp.concatenate(rows, axis=0), mf[g], preferred_element_type=f32)
            for par in range(2):
                sig[par] += [o[par * P:(par + 1) * P, :128], o[par * P:(par + 1) * P, 128:]]
        y0, y1 = _merge8(sig[0]), _merge8(sig[1])
        for t in range(8):
            bx[j, :, t * 128:(t + 1) * 128] = pltpu.pack_elementwise([y0[t], y1[t]], packed_dtype=bf16)
        return carry

    lax.fori_loop(0, R // 2, inv, 0)

    row = lax.broadcasted_iota(jnp.int32, (L, L), 0)
    col = lax.broadcasted_iota(jnp.int32, (L, L), 1)
    mask = (row < M) | (row >= col)
    scale = np.float32(DH ** -0.5)
    wsplit = wqkv.reshape(3 * (H // 2), D // 16, 16, 128)

    def out_copy(s):
        return pltpu.make_async_copy(oa.at[pl.ds(2 * s, 2)], out_hbm.at[pl.ds(2 * s, 2), :, pl.ds(0, D)], sem_out.at[0])

    def load_tokens(slot, u):
        hbuf[M:L, :] = ax[slot, u * SEG:(u + 1) * SEG, :].astype(f32)

    def proj(j, par, slot):
        for m in range(3):
            w = wsplit[m * (H // 2) + j, :, 8 * par:8 * par + 8, :].reshape(D // 2, 128)
            qkv[slot, m] = jnp.dot(hbuf[...], pltpu.bitcast(w, bf16), preferred_element_type=f32)

    def proj_split(j, par, slot):
        for half in range(2):
            for m in range(3):
                w = wsplit[m * (H // 2) + j, 32 * half:32 * half + 32, 8 * par:8 * par + 8, :].reshape(D // 4, 128)
                o = jnp.dot(hbuf[:, half * (D // 2):(half + 1) * (D // 2)], pltpu.bitcast(w, bf16),
                            preferred_element_type=f32)
                qkv[slot, m] = o if half == 0 else qkv[slot, m] + o

    def scores(slot):
        sc = _nt(qkv[slot, 0], qkv[slot, 1]) * scale
        sc = jnp.where(mask, sc, -1e9)
        e = jnp.exp(sc - jnp.max(sc, axis=-1, keepdims=True))
        pbuf[slot % 4] = e / jnp.sum(e, axis=-1, keepdims=True)

    def pv(h, slot):
        obuf[h] = jnp.dot(pbuf[slot % 4], qkv[slot, 2], preferred_element_type=f32)

    def oproj(c, h0, h1):
        o = jnp.concatenate([obuf[h] for h in range(h0, h1)], axis=1)
        return jnp.dot(o, pltpu.bitcast(wo[c, 64 * h0:64 * h1, :], bf16), preferred_element_type=f32)

    def finish(s, c, o):
        hbuf[0:M, 128 * c:128 * (c + 1)] = o[0:M].astype(bf16).astype(f32)
        oa[pl.ds(2 * s, 2), :, 128 * c:128 * (c + 1)] = o[M:L].astype(bf16).reshape(2, R, 128)

    mem_copy.wait()
    ax0_copy.wait()
    ax_copy(0).start()
    hbuf[0:M, :] = mem_ref[...].astype(f32)
    load_tokens(1, 0)

    def first(j, carry):
        for cp in qkv_copies(j):
            cp.wait()

        def split(g, carry):
            jj = (g // 4) * (H // 2) + j
            base = pl.multiple_of((g % 4) * 256, 256)
            ev = [wqkv[jj, pl.ds(base + 16 * i, 8, stride=2), :] for i in range(16)]
            od = [wqkv[jj, pl.ds(base + 16 * i + 1, 8, stride=2), :] for i in range(16)]
            for i in range(16):
                wqkv[jj, pl.ds(base + 16 * i, 8), :] = (ev[i] & 0xFFFF) | (od[i] << 16)
                wqkv[jj, pl.ds(base + 16 * i + 8, 8), :] = (ev[i] >> 16) | (od[i] & jnp.uint32(0xFFFF0000))
            return carry

        lax.fori_loop(0, 12, split, 0)
        for par in range(2):
            proj(j, par, par)
        for par in range(2):
            scores(par)
        for par in range(2):
            pv(2 * j + par, par)
        return carry

    lax.fori_loop(0, H // 2, first, 0)
    for c in range(D // 128):
        wo_copies[c].wait()
        finish(0, c, oproj(c, 0, H))
    out_copy(0).start()
    for j in range(R // 2):
        y_copy(j).start()

    def seg(s):
        for g in range(H // 4):
            prev = range(4 * g - 4, 4 * g) if g else ()
            (proj if g else proj_split)(2 * g, 0, (4 * g) % 8)
            for h in prev:
                scores(h % 8)
            for h in range(4 * g + 1, 4 * g + 4):
                proj(h // 2, h % 2, h % 8)
            for h in prev:
                pv(h, h % 8)
        part[0] = oproj(0, 0, 24)
        for h in range(H - 4, H):
            scores(h % 8)
        part[1] = oproj(1, 0, 28)
        part[2] = oproj(2, 0, 28)
        for h in range(H - 4, H):
            pv(h, h % 8)
        part[3] = oproj(3, 0, 28)
        finish(s, 0, part[0] + oproj(0, 24, 32))
        for c in range(1, 4):
            finish(s, c, part[c] + oproj(c, 28, 32))
        for c in range(4, 8):
            finish(s, c, oproj(c, 0, 32))

    def trip(t, carry):
        ax_copy(t).wait()
        ax_copy(t + 1).start()
        for u in range(UNROLL):
            load_tokens(t % 2, u)
            seg(1 + UNROLL * t + u)
        for u in range(UNROLL):
            out_copy(1 + UNROLL * t + u).start()
        return carry

    lax.fori_loop(0, NTRIP, trip, 0)
    ax_copy(NTRIP).wait()

    def drain(s, carry):
        out_copy(s).wait()
        return carry

    lax.fori_loop(0, NSEG, drain, 0)
    for j in range(R // 2):
        y_copy(j).wait()


@functools.partial(jax.jit, static_argnames=("A_seg_len",))
def pallas_concat_heads__memory_aug_recurrent_mem_tr__spectral_gfnet__prompt_kernel(
    A_x, A_mem0, A_Wq, A_Wk, A_Wv, A_Wo, A_seg_len, B_x, B_w_r, B_w_i,
):
    assert A_seg_len == SEG and A_x.shape == (1, S, D) and B_x.shape == (1, S, D)
    mf, tab = _constants()
    hbm = pl.BlockSpec(memory_space=pltpu.HBM)
    nyq = pl.BlockSpec((8, S), lambda i: (D // 16, 0))
    wr, wi = B_w_r.T, B_w_i.T
    out = pl.pallas_call(
        _kernel,
        out_shape=jax.ShapeDtypeStruct((P, R, 2 * D), bf16),
        grid=(1,),
        in_specs=[hbm] * 9 + [nyq, nyq] + [hbm] * 2,
        out_specs=hbm,
        scratch_shapes=[
            pltpu.VMEM((3 * H // 2, D, 128), u32),
            pltpu.VMEM((D // 128, H * DH // 2, 128), u32),
            pltpu.VMEM((2, UNROLL * SEG, D), bf16),
            pltpu.VMEM((P, R, D), bf16),
            pltpu.VMEM((R // 2, P, D), u32),
            pltpu.VMEM((NT, 256, 256), bf16),
            pltpu.VMEM((4, P, P), f32),
            pltpu.VMEM((R, 2 * P, 2 * P), bf16),
            pltpu.VMEM((R, D // 4, P), u32),
            pltpu.VMEM((R, D // 4, P), u32),
            pltpu.VMEM((R, D // 2 + 8, 2 * P), f32),
            pltpu.VMEM((M, D), bf16),
            pltpu.VMEM((L, D), f32),
            pltpu.VMEM((H, L, DH), f32),
            pltpu.VMEM((8, 3, L, DH), f32),
            pltpu.VMEM((4, L, L), f32),
            pltpu.VMEM((4, L, 128), f32),
            pltpu.SemaphoreType.DMA((R // 2,)),
            pltpu.SemaphoreType.DMA((H // 2,)),
            pltpu.SemaphoreType.DMA((D // 128,)),
            pltpu.SemaphoreType.DMA((12,)),
            pltpu.SemaphoreType.DMA((1,)),
        ],
        compiler_params=pltpu.CompilerParams(vmem_limit_bytes=110 * 2**20),
        name="rmt_gfnet",
    )(A_x.reshape(S, D), A_mem0.reshape(M, D), A_Wq, A_Wk, A_Wv, A_Wo.reshape(H * DH, D),
      B_x.reshape(P, R, D), wr, wi, wr, wi, mf, tab)
    return out.reshape(1, S, 2 * D)
```

```python
import functools

import jax
import jax.numpy as jnp
import numpy as np
from jax import lax
import jax.experimental.pallas as pl
import jax.experimental.pallas.tpu as pltpu

f32, bf16, u32 = jnp.float32, jnp.bfloat16, jnp.uint32

S, D = 2048, 1024
H, DH, M, SEG = 32, 128, 8, 32
L = M + SEG
NSEG = S // SEG
UNROLL = 3
NTRIP = (NSEG - 1) // UNROLL
R, P = 16, 128
NT = D // 2 // 128


_RT = float(np.sqrt(0.5))


def _split8(x):
    a0, a1, b0, b1 = x[0] + x[4], x[0] - x[4], x[2] + x[6], x[2] - x[6]
    c0, c1, d0, d1 = x[1] + x[5], x[1] - x[5], x[3] + x[7], x[3] - x[7]
    e, f = a0 + b0, c0 + d0
    u, v = (c1 - d1) * _RT, (c1 + d1) * _RT
    return [e + f, e - f, a1 + u, b1 + v, a0 - b0, c0 - d0, a1 - u, b1 - v]


def _merge8(y):
    e, f = y[0] + y[1], y[0] - y[1]
    a0, b0, c0, d0 = e + y[4], e - y[4], f + y[5], f - y[5]
    a1, b1 = y[2] + y[6], y[3] + y[7]
    u, v = (y[2] - y[6]) * _RT, (y[3] - y[7]) * _RT
    c1, d1 = u + v, v - u
    return [a0 + a1, c0 + c1, b0 + b1, d0 + d1, a0 - a1, c0 - c1, b0 - b1, d0 - d1]


_GROUPS = ((0, 4), (1, 7), (2, 6), (3, 5))


@functools.lru_cache(maxsize=None)
def _constants():
    basis = np.stack(_split8(list(np.eye(8))))
    d = np.arange(D)[None, :]
    mf = []
    for g, ks in enumerate(_GROUPS):
        kd = np.sort(np.concatenate([k1 + 8 * np.arange(64) for k1 in ks]))[:, None]
        ang = 2.0 * np.pi * ((d * kd) % D) / D
        rows = np.concatenate([np.cos(ang), -np.sin(ang)], axis=0)
        if g == 0:
            rows[128] = 1.0 - 2.0 * (np.arange(D) % 2)
        bg = basis[2 * g:2 * g + 2]
        rows = rows.reshape(256, 8, 128)
        m = np.einsum("oad,as->osd", rows, np.linalg.pinv(bg))
        assert np.abs(np.einsum("osd,sa->oad", m, bg) - rows).max() < 1e-9
        mf.append(m.reshape(256, 256))
    k2 = np.arange(P)[None, :]
    a = 2.0 * np.pi * ((np.arange(P)[:, None] * k2) % P) / P
    t = 2.0 * np.pi * (np.repeat(np.arange(R), 8)[:, None] * k2) / S
    tab = np.stack([np.cos(a), -np.sin(a), np.cos(t) * 2.0 ** -10, -np.sin(t) * 2.0 ** -10])
    return np.stack(mf).astype(bf16), tab.astype(np.float32)


def _fft16(xs, sign):
    def bf4(a, b, c, d):
        s0 = (a[0] + c[0], a[1] + c[1])
        s1 = (a[0] - c[0], a[1] - c[1])
        s2 = (b[0] + d[0], b[1] + d[1])
        s3 = (b[0] - d[0], b[1] - d[1])
        p = (s1[0] - s3[1], s1[1] + s3[0])
        m = (s1[0] + s3[1], s1[1] - s3[0])
        o1, o3 = (p, m) if sign > 0 else (m, p)
        return [(s0[0] + s2[0], s0[1] + s2[1]), o1, (s0[0] - s2[0], s0[1] - s2[1]), o3]

    def tw(x, e):
        e = e % 16
        if e == 0:
            return x
        if e == 4:
            return (-x[1], x[0]) if sign > 0 else (x[1], -x[0])
        c = np.float32(np.cos(2 * np.pi * e / 16))
        s = np.float32(sign * np.sin(2 * np.pi * e / 16))
        if e == 2:
            return ((x[0] - x[1]) * c, (x[0] + x[1]) * c) if sign > 0 else ((x[0] + x[1]) * c, (x[1] - x[0]) * c)
        if e == 6:
            return ((x[0] + x[1]) * c, (x[1] - x[0]) * c) if sign > 0 else ((x[0] - x[1]) * c, (x[0] + x[1]) * c)
        return (x[0] * c - x[1] * s, x[0] * s + x[1] * c)

    inner = [bf4(xs[b], xs[4 + b], xs[8 + b], xs[12 + b]) for b in range(4)]
    out = [None] * 16
    for c in range(4):
        o = bf4(*[tw(inner[b][c], b * c) for b in range(4)])
        for e in range(4):
            out[c + 4 * e] = o[e]
    return out


def _nt(a, b):
    return lax.dot_general(a, b, (((1,), (1,)), ((), ())), preferred_element_type=f32)


def _kernel(ax_hbm, mem_hbm, wq_hbm, wk_hbm, wv_hbm, wo_hbm, bx_hbm, wr_hbm, wi_hbm, wrn_ref, win_ref,
            mf_hbm, tab_hbm, out_hbm,
            wqkv, wo, ax, oa, bx, mf, tab, gf, wr, wi, tp, mem_ref,
            hbuf, obuf, qkv, pbuf, part, sem_bx, sem_qkv, sem_wo, sem, sem_out):
    bx32 = bx_hbm.bitcast(u32)
    out32 = out_hbm.bitcast(u32)

    def bx_copy(j):
        return pltpu.make_async_copy(bx32.at[:, j, :], bx.at[j], sem_bx.at[j])

    def y_copy(j):
        return pltpu.make_async_copy(bx.at[j], out32.at[:, j, pl.ds(D, D)], sem.at[10])

    mf_copy = pltpu.make_async_copy(mf_hbm, mf, sem.at[0])
    tab_copy = pltpu.make_async_copy(tab_hbm, tab, sem.at[1])

    ax0_copy = pltpu.make_async_copy(ax_hbm.at[pl.ds(0, SEG), :], ax.at[1, pl.ds(0, SEG), :], sem.at[2])

    def ax_copy(t):
        r0 = pl.multiple_of(SEG + jnp.minimum(t, NTRIP - 1) * (UNROLL * SEG), SEG)
        return pltpu.make_async_copy(ax_hbm.at[pl.ds(r0, UNROLL * SEG), :], ax.at[t % 2], sem.at[2])

    mem_copy = pltpu.make_async_copy(mem_hbm, mem_ref, sem.at[11])
    w_copies = [pltpu.make_async_copy(src.at[pl.ds(0, D // 2), pl.ds(k1 * P, P)].bitcast(u32), dst.at[k1], sem.at[5])
                for src, dst in ((wr_hbm, wr), (wi_hbm, wi)) for k1 in range(R)]

    def qkv_copies(j):
        return [pltpu.make_async_copy(src.bitcast(u32).at[:, j, :], wqkv.at[m * (H // 2) + j], sem_qkv.at[j])
                for m, src in enumerate((wq_hbm, wk_hbm, wv_hbm))]

    wo32 = wo_hbm.bitcast(u32)
    wo_copies = [pltpu.make_async_copy(wo32.at[:, pl.ds(c * 128, 128)], wo.at[c], sem_wo.at[c]) for c in range(D // 128)]

    mf_copy.start()
    bx_copy(0).start()
    tab_copy.start()
    for j in range(1, R // 2):
        bx_copy(j).start()
    for cp in w_copies:
        cp.start()
    mem_copy.start()
    ax0_copy.start()

    def unpack(w, par):
        return pltpu.bitcast((w << 16) if par == 0 else (w & jnp.uint32(0xFFFF0000)), f32)

    mf_copy.wait()
    tab_copy.wait()
    row0 = lax.broadcasted_iota(jnp.int32, (8, 128), 0) == 0

    def fwd(j, carry):
        bx_copy(j).wait()

        @pl.when(j == 5)
        def _():
            for jj in range(H // 2):
                for cp in qkv_copies(jj):
                    cp.start()

        zs = []
        for par in range(2):
            sig = _split8([unpack(bx[j, :, t * 128:(t + 1) * 128], par) for t in range(8)])
            zs.append([_nt(mf[g], jnp.concatenate([sig[2 * g].astype(bf16), sig[2 * g + 1].astype(bf16)], axis=1))
                       for g in range(NT)])
        for par in range(2):
            z = zs[par]
            head = z[0][128:136]
            re = [zg[:128] for zg in z] + [jnp.where(row0, head, 0.0)]
            im = [jnp.where(row0, 0.0, head), z[0][136:]] + [zg[128:] for zg in z[1:]] + [jnp.zeros((8, 128), f32)]
            lhs = jnp.concatenate([jnp.concatenate(re, axis=0), jnp.concatenate(im, axis=0)], axis=1)
            n1 = 2 * j + par
            tr = jnp.tile(tab[2, pl.ds(pl.multiple_of(8 * n1, 8), 8), :], (P // 8, 1))
            ti = jnp.tile(tab[3, pl.ds(pl.multiple_of(8 * n1, 8), 8), :], (P // 8, 1))
            gr, gi = tab[0] * tr - tab[1] * ti, tab[0] * ti + tab[1] * tr
            gm = jnp.concatenate([jnp.concatenate([gr, gi], axis=1),
                                  jnp.concatenate([-gi, gr], axis=1)], axis=0).astype(bf16)
            gf[n1] = gm
            tp[n1] = jnp.dot(lhs, gm, preferred_element_type=f32)
        return carry

    lax.fori_loop(0, R // 2, fwd, 0)

    for cp in w_copies:
        cp.wait()

    def filt(r0, w_of):
        xs = _fft16([(tp[n1, pl.ds(r0, 8), :P], tp[n1, pl.ds(r0, 8), P:]) for n1 in range(R)], -1)
        ys = []
        for k1, (ur, ui) in enumerate(xs):
            a, b = w_of(k1)
            ys.append((ur * a - ui * b, ur * b + ui * a))
        for n1, (yr, yi) in enumerate(_fft16(ys, 1)):
            tp[n1, pl.ds(r0, 8), :P] = yr
            tp[n1, pl.ds(r0, 8), P:] = yi

    even = lax.broadcasted_iota(jnp.int32, (8, 128), 0) % 2 == 0
    for g in range(NT):
        def body(i, carry, g=g):
            def w_of(k1):
                def rows(ref):
                    def ld(q):
                        return ref[k1, pl.ds(16 * i + q, 8, stride=2), :]
                    if g % 2 == 0:
                        return unpack(ld(g // 2), 0)
                    return unpack(jnp.where(even, ld(g // 2), ld(1 - g // 2)), 1)
                a, b = rows(wr), rows(wi)
                if g == 0:
                    half0 = jnp.where(row0 & (i == 0), 0.5, 1.0)
                    a, b = a * half0, b * half0
                return a, b
            filt(pl.multiple_of(g * 128 + 8 * i, 8), w_of)
            return carry
        lax.fori_loop(0, 16, body, 0)
    filt(D // 2, lambda k1: (jnp.where(row0, wrn_ref[:, k1 * P:(k1 + 1) * P].astype(f32), 0.0) * 0.5,
                             jnp.where(row0, win_ref[:, k1 * P:(k1 + 1) * P].astype(f32), 0.0) * 0.5))

    for cp in wo_copies:
        cp.start()
    lane0 = lax.broadcasted_iota(jnp.int32, (P, 128), 1) == 0

    def inv(j, carry):
        ts = []
        for par in range(2):
            n1 = 2 * j + par
            ts.append([_nt(gf[n1], tp[n1, t * 128:(t + 1) * 128, :].astype(bf16)) for t in range(NT)])
        for par in range(2):
            n1 = 2 * j + par
            ny = jnp.concatenate([tp[n1, D // 2:, :], jnp.zeros((120, 2 * P), f32)], axis=0)
            ts[par].append(_nt(gf[n1, :P, :], ny.astype(bf16)))
        sig = [[], []]
        for g in range(NT):
            rows = []
            for par in range(2):
                t = ts[par][g]
                ti = jnp.where(lane0, ts[par][NT], t[P:]) if g == 0 else t[P:]
                rows.append(jnp.concatenate([t[:P], ti], axis=1))
            o = jnp.dot(jnp.concatenate(rows, axis=0), mf[g], preferred_element_type=f32)
            for par in range(2):
                sig[par] += [o[par * P:(par + 1) * P, :128], o[par * P:(par + 1) * P, 128:]]
        y0, y1 = _merge8(sig[0]), _merge8(sig[1])
        for t in range(8):
            lo, hi = (pltpu.bitcast(y[t].astype(bf16).astype(f32), u32) for y in (y0, y1))
            bx[j, :, t * 128:(t + 1) * 128] = (lo >> 16) | hi
        return carry

    lax.fori_loop(0, R // 2, inv, 0)

    row = lax.broadcasted_iota(jnp.int32, (L, L), 0)
    col = lax.broadcasted_iota(jnp.int32, (L, L), 1)
    mask = (row < M) | (row >= col)
    scale = np.float32(DH ** -0.5)
    wsplit = wqkv.reshape(3 * (H // 2), D // 16, 16, 128)

    def out_copy(s):
        return pltpu.make_async_copy(oa.at[pl.ds(2 * s, 2)], out_hbm.at[pl.ds(2 * s, 2), :, pl.ds(0, D)], sem_out.at[0])

    def load_tokens(slot, u):
        hbuf[M:L, :] = ax[slot, u * SEG:(u + 1) * SEG, :].astype(f32)

    def proj(j, par, slot):
        for m in range(3):
            w = wsplit[m * (H // 2) + j, :, 8 * par:8 * par + 8, :].reshape(D // 2, 128)
            qkv[slot, m] = jnp.dot(hbuf[...], pltpu.bitcast(w, bf16), preferred_element_type=f32)

    def proj_split(j, par, slot):
        for half in range(2):
            for m in range(3):
                w = wsplit[m * (H // 2) + j, 32 * half:32 * half + 32, 8 * par:8 * par + 8, :].reshape(D // 4, 128)
                o = jnp.dot(hbuf[:, half * (D // 2):(half + 1) * (D // 2)], pltpu.bitcast(w, bf16),
                            preferred_element_type=f32)
                qkv[slot, m] = o if half == 0 else qkv[slot, m] + o

    def scores(slot):
        sc = _nt(qkv[slot, 0], qkv[slot, 1]) * scale
        sc = jnp.where(mask, sc, -1e9)
        e = jnp.exp(sc - jnp.max(sc, axis=-1, keepdims=True))
        pbuf[slot % 4] = e / jnp.sum(e, axis=-1, keepdims=True)

    def pv(h, slot):
        obuf[h] = jnp.dot(pbuf[slot % 4], qkv[slot, 2], preferred_element_type=f32)

    def oproj(c, h0, h1):
        o = jnp.concatenate([obuf[h] for h in range(h0, h1)], axis=1)
        return jnp.dot(o, pltpu.bitcast(wo[c, 64 * h0:64 * h1, :], bf16), preferred_element_type=f32)

    def finish(s, c, o):
        hbuf[0:M, 128 * c:128 * (c + 1)] = o[0:M].astype(bf16).astype(f32)
        oa[pl.ds(2 * s, 2), :, 128 * c:128 * (c + 1)] = o[M:L].astype(bf16).reshape(2, R, 128)

    mem_copy.wait()
    ax0_copy.wait()
    ax_copy(0).start()
    hbuf[0:M, :] = mem_ref[...].astype(f32)
    load_tokens(1, 0)

    def first(j, carry):
        for cp in qkv_copies(j):
            cp.wait()

        def split(g, carry):
            jj = (g // 4) * (H // 2) + j
            base = pl.multiple_of((g % 4) * 256, 256)
            ev = [wqkv[jj, pl.ds(base + 16 * i, 8, stride=2), :] for i in range(16)]
            od = [wqkv[jj, pl.ds(base + 16 * i + 1, 8, stride=2), :] for i in range(16)]
            for i in range(16):
                wqkv[jj, pl.ds(base + 16 * i, 8), :] = (ev[i] & 0xFFFF) | (od[i] << 16)
                wqkv[jj, pl.ds(base + 16 * i + 8, 8), :] = (ev[i] >> 16) | (od[i] & jnp.uint32(0xFFFF0000))
            return carry

        lax.fori_loop(0, 12, split, 0)
        for par in range(2):
            proj(j, par, par)
        for par in range(2):
            scores(par)
        for par in range(2):
            pv(2 * j + par, par)
        return carry

    lax.fori_loop(0, H // 2, first, 0)
    for c in range(D // 128):
        wo_copies[c].wait()
        finish(0, c, oproj(c, 0, H))
    for j in range(R // 2):
        y_copy(j).start()

    def seg(s):
        for g in range(H // 4):
            prev = range(4 * g - 4, 4 * g) if g else ()
            (proj if g else proj_split)(2 * g, 0, (4 * g) % 8)
            for h in prev:
                scores(h % 8)
            for h in range(4 * g + 1, 4 * g + 4):
                proj(h // 2, h % 2, h % 8)
            for h in prev:
                pv(h, h % 8)
        part[0] = oproj(0, 0, 24)
        for h in range(H - 4, H):
            scores(h % 8)
        part[1] = oproj(1, 0, 28)
        part[2] = oproj(2, 0, 28)
        for h in range(H - 4, H):
            pv(h, h % 8)
        part[3] = oproj(3, 0, 28)
        finish(s, 0, part[0] + oproj(0, 24, 32))
        for c in range(1, 4):
            finish(s, c, part[c] + oproj(c, 28, 32))
        for c in range(4, 8):
            finish(s, c, oproj(c, 0, 32))

    def trip(t, carry):
        for u in range(UNROLL):
            s = 1 + UNROLL * t + u
            seg(s)
            if u == 0:
                out_copy(s - 1).start()
                ax_copy(t + 1).start()
            else:
                out_copy(s - 1).start()
            if u + 1 < UNROLL:
                load_tokens(t % 2, u + 1)
            else:
                ax_copy(t + 1).wait()
                load_tokens((t + 1) % 2, 0)
        return carry

    ax_copy(0).wait()
    load_tokens(0, 0)
    lax.fori_loop(0, NTRIP, trip, 0)
    out_copy(NSEG - 1).start()

    def drain(s, carry):
        out_copy(s).wait()
        return carry

    lax.fori_loop(0, NSEG, drain, 0)
    for j in range(R // 2):
        y_copy(j).wait()


@functools.partial(jax.jit, static_argnames=("A_seg_len",))
def pallas_concat_heads__memory_aug_recurrent_mem_tr__spectral_gfnet__prompt_kernel(
    A_x, A_mem0, A_Wq, A_Wk, A_Wv, A_Wo, A_seg_len, B_x, B_w_r, B_w_i,
):
    assert A_seg_len == SEG and A_x.shape == (1, S, D) and B_x.shape == (1, S, D)
    mf, tab = _constants()
    hbm = pl.BlockSpec(memory_space=pltpu.HBM)
    nyq = pl.BlockSpec((8, S), lambda i: (D // 16, 0))
    wr, wi = B_w_r.T, B_w_i.T
    out = pl.pallas_call(
        _kernel,
        out_shape=jax.ShapeDtypeStruct((P, R, 2 * D), bf16),
        grid=(1,),
        in_specs=[hbm] * 9 + [nyq, nyq] + [hbm] * 2,
        out_specs=hbm,
        scratch_shapes=[
            pltpu.VMEM((3 * H // 2, D, 128), u32),
            pltpu.VMEM((D // 128, H * DH // 2, 128), u32),
            pltpu.VMEM((2, UNROLL * SEG, D), bf16),
            pltpu.VMEM((P, R, D), bf16),
            pltpu.VMEM((R // 2, P, D), u32),
            pltpu.VMEM((NT, 256, 256), bf16),
            pltpu.VMEM((4, P, P), f32),
            pltpu.VMEM((R, 2 * P, 2 * P), bf16),
            pltpu.VMEM((R, D // 4, P), u32),
            pltpu.VMEM((R, D // 4, P), u32),
            pltpu.VMEM((R, D // 2 + 8, 2 * P), f32),
            pltpu.VMEM((M, D), bf16),
            pltpu.VMEM((L, D), f32),
            pltpu.VMEM((H, L, DH), f32),
            pltpu.VMEM((8, 3, L, DH), f32),
            pltpu.VMEM((4, L, L), f32),
            pltpu.VMEM((4, L, 128), f32),
            pltpu.SemaphoreType.DMA((R // 2,)),
            pltpu.SemaphoreType.DMA((H // 2,)),
            pltpu.SemaphoreType.DMA((D // 128,)),
            pltpu.SemaphoreType.DMA((12,)),
            pltpu.SemaphoreType.DMA((1,)),
        ],
        compiler_params=pltpu.CompilerParams(vmem_limit_bytes=110 * 2**20),
        name="rmt_gfnet",
    )(A_x.reshape(S, D), A_mem0.reshape(M, D), A_Wq, A_Wk, A_Wv, A_Wo.reshape(H * DH, D),
      B_x.reshape(P, R, D), wr, wi, wr, wi, mf, tab)
    return out.reshape(1, S, 2 * D)
```
